```python
import jax
import jax.numpy as jnp

def _softmax(x, axis=-1):
    return jax.nn.softmax(x, axis=axis)
def _gelu(x):
    return jax.nn.gelu(x, approximate=True)
def _silu(x):
    return jax.nn.silu(x)
def _sigmoid(x):
    return jax.nn.sigmoid(x)
def _layernorm(x, axis=-1, eps=1e-5):
    m = jnp.mean(x, axis=axis, keepdims=True)
    v = jnp.var(x, axis=axis, keepdims=True)
    return (x - m) / jnp.sqrt(v + eps)
def _scatter_add(tgt, idx, src, axis=0):
    return tgt.at[idx].add(src)
def _segment_sum(src, seg, n):
    return jax.ops.segment_sum(src, seg, n)
class _Rng:
    def __init__(self, key):
        self._k = key
    def _next(self):
        self._k, sub = jax.random.split(self._k)
        return sub
    def normal(self, shape):
        return jax.random.normal(self._next(), shape, dtype=jnp.bfloat16)
    def randint(self, lo, hi, shape):
        return jax.random.randint(self._next(), shape, lo, hi, dtype=jnp.int32)
    def uniform(self, shape, lo=0.0, hi=1.0):
        return jax.random.uniform(self._next(), shape, jnp.bfloat16, lo, hi)
    def permutation(self, n):
        return jax.random.permutation(self._next(), n)


kernel_name = 'parallel_sum__linear_attn_block__moe_arch_mod__prompt'

def setup_inputs():
    _rng = _Rng(jax.random.key(int.from_bytes(__import__("os").urandom(4), "little")))
    _w = (lambda a: (lambda t: t.astype(jnp.bfloat16) if jnp.issubdtype(t.dtype, jnp.floating) else t)(jnp.asarray(a)))
    def _A_setup():
        B, S, D = 1, 2048, 1024
        return {
            "x": _w((lambda *s: _rng.normal(s) * 0.05)(B, S, D)),
            "wqkv": _w((lambda *s: _rng.normal(s) * 0.05)(D, 3 * D)),
            "wo": _w((lambda *s: _rng.normal(s) * 0.05)(D, D)),
        }
    _A_in = _A_setup()

    def _B_setup():
        B, S, D, F, C = 1, 2048, 1024, 3584, 1
        return {
            "x": _w((lambda *s: _rng.normal(s) * 0.05)(B, S, D)),
            "w_r": _w((lambda *s: _rng.normal(s) * 0.05)(D)),
            "w_gate": _w((lambda *s: _rng.normal(s) * 0.05)(D, F)),
            "w_up": _w((lambda *s: _rng.normal(s) * 0.05)(D, F)),
            "w_down": _w((lambda *s: _rng.normal(s) * 0.05)(F, D)),
        }
    _B_in = _B_setup()

    return {
        "A_x": _A_in["x"],
        "A_wqkv": _A_in["wqkv"],
        "A_wo": _A_in["wo"],
        "B_x": _B_in["x"],
        "B_w_r": _B_in["w_r"],
        "B_w_gate": _B_in["w_gate"],
        "B_w_up": _B_in["w_up"],
        "B_w_down": _B_in["w_down"],
    }

def reference(A_x, A_wqkv, A_wo, B_x, B_w_r, B_w_gate, B_w_up, B_w_down):
    def _A_ref(x, wqkv, wo):
        B, S, D = x.shape
        H = 32; Dh = D // H
        qkv = (lambda x, *d: x.transpose(*d))((x @ wqkv).reshape(B, S, 3, H, Dh), 2, 0, 3, 1, 4)
        q, k, v = qkv[0], qkv[1], qkv[2]
        phi = lambda t: jnp.where(t > 0, t + 1, jnp.exp(t)) + 1e-6
        pq, pk = phi(q), phi(k)
        kv = jnp.einsum("bhsd,bhse->bhde", pk, v)
        z = jnp.einsum("bhsd->bhd", pk)
        num = jnp.einsum("bhqd,bhde->bhqe", pq, kv)
        den = jnp.einsum("bhqd,bhd->bhq", pq, z)[..., None] + 1e-6
        o = num / den
        return (lambda x, *d: x.transpose(*d))(o, 0, 2, 1, 3).reshape(B, S, D) @ wo

    def _B_ref(x, w_r, w_gate, w_up, w_down):
        B, S, D = x.shape
        C = 1
        r = x @ w_r
        idx = jnp.argsort(-r, axis=-1)[:, :C]
        idx_e = jnp.repeat(idx.reshape(B, C, 1), D, axis=2)
        x_sel = jnp.take_along_axis(x, idx_e, axis=1)
        g = _silu(x_sel @ w_gate)
        u = x_sel @ w_up
        y = (g * u) @ w_down
        r_sel = _sigmoid(jnp.take_along_axis(r, idx, axis=1))
        y = y * r_sel.reshape(B, C, 1)
        b_off = (jnp.arange(B) * S).reshape(B, 1)
        flat_idx = (idx + b_off).reshape(B * C)
        zero = (x * 0.0).reshape(B * S, D)
        upd = _scatter_add(zero, flat_idx, y.reshape(B * C, D), axis=0)
        return x + upd.reshape(B, S, D)

    x = A_x
    xn = _layernorm(x, axis=-1)
    return x + _A_ref(xn, A_wqkv, A_wo) + _B_ref(xn, B_w_r, B_w_gate, B_w_up, B_w_down)
```

```python
import functools
import numpy as np
import jax
import jax.numpy as jnp
from jax import lax
from jax.experimental import pallas as pl
from jax.experimental.pallas import tpu as pltpu

S, D, H, DH, F = 2048, 1024, 32, 32, 3584
G = D // 128
f32, bf16 = jnp.float32, jnp.bfloat16
EPS_B = 1.00135803e-05


def _rb(x):
    return x.astype(bf16).astype(f32)


def _phi(t):
    return jnp.where(t > 0, t + 1.0, jnp.exp(t)) + 1e-6


def make_kernel(TM=512, CR=64):
    NB = S // TM
    CH = F // NB
    assert CH % 128 == 0

    def kernel(x_hbm, wqkv_hbm, wo_hbm, wr_hbm, wg_hbm, wu_hbm, wd_hbm, out_hbm,
               x_v, xn_v, wq_v, wk_v, wv_v, wo_v, m_v, wr_v, wg_v, wu_v, wd_v,
               kv_v, z_v, zt_v, r_v, op_v, out_v, y_v,
               x_sem, w_sem, g_sem, u_sem, d_sem, o_sem, p_sem):
        def x_cp(i):
            r0 = pl.multiple_of(i * TM, TM) if not isinstance(i, int) else i * TM
            return pltpu.make_async_copy(x_hbm.at[pl.ds(r0, TM), :], x_v.at[pl.ds(r0, TM), :], x_sem.at[i])
        wq_cp = pltpu.make_async_copy(wqkv_hbm.at[:, pl.ds(0, D)], wq_v, w_sem.at[0])
        wk_cp = pltpu.make_async_copy(wqkv_hbm.at[:, pl.ds(D, D)], wk_v, w_sem.at[1])
        wv_cp = pltpu.make_async_copy(wqkv_hbm.at[:, pl.ds(2 * D, D)], wv_v, w_sem.at[2])
        wo_cp = pltpu.make_async_copy(wo_hbm, wo_v, w_sem.at[3])
        wr_cp = pltpu.make_async_copy(wr_hbm, wr_v, w_sem.at[4])
        def g_cp(c):
            c0 = pl.multiple_of(c * CH, 128) if not isinstance(c, int) else c * CH
            return pltpu.make_async_copy(wg_hbm.at[:, pl.ds(c0, CH)], wg_v.at[:, pl.ds(c0, CH)], g_sem.at[c])
        def u_cp(c):
            c0 = pl.multiple_of(c * CH, 128) if not isinstance(c, int) else c * CH
            return pltpu.make_async_copy(wu_hbm.at[:, pl.ds(c0, CH)], wu_v.at[:, pl.ds(c0, CH)], u_sem.at[c])
        def d_cp(c):
            c0 = pl.multiple_of(c * CH, 128) if not isinstance(c, int) else c * CH
            return pltpu.make_async_copy(wd_hbm.at[pl.ds(c0, CH), :], wd_v.at[pl.ds(c0, CH), :], d_sem.at[c])
        def o_cp(i):
            r0 = pl.multiple_of(i * TM, TM) if not isinstance(i, int) else i * TM
            return pltpu.make_async_copy(out_v.at[pl.ds(r0, TM), :], out_hbm.at[pl.ds(r0, TM), :], o_sem.at[i])

        x_cp(0).start()
        wr_cp.start()
        wk_cp.start()
        wv_cp.start()

        wr_cp.wait()
        wr = wr_v[...].astype(f32).reshape(1, D)

        def ln_block(i):
            r0 = pl.multiple_of(i * TM, TM) if not isinstance(i, int) else i * TM
            for c in range(TM // CR):
                rows = pl.ds(r0 + c * CR, CR)
                xf = x_v[rows, :].astype(f32)
                mean = jnp.sum(xf, axis=1, keepdims=True) * (1.0 / D)
                mb = _rb(mean)
                d = xf - mb
                dm = mean - mb
                var = jnp.sum(d * d, axis=1, keepdims=True) * (1.0 / D) - dm * dm
                s = _rb(jnp.sqrt(_rb(_rb(var) + EPS_B)))
                xn_b = (_rb(d) * (1.0 / s)).astype(bf16)
                xn_v[rows, :] = xn_b
                r = jnp.sum(xn_b.astype(f32) * wr, axis=1, keepdims=True)
                r_v[rows, :] = _rb(r)

        kv_v[...] = jnp.zeros_like(kv_v)
        z_v[...] = jnp.zeros_like(z_v)
        x_cp(0).wait()
        ln_block(0)
        for i in range(1, NB):
            x_cp(i).start()
        wk_cp.wait()
        wv_cp.wait()
        wq_cp.start()
        wo_cp.start()

        def pass1(i, carry):
            g_cp(i).start()
            u_cp(i).start()
            d_cp(i).start()
            nxt = jnp.minimum(i + 1, NB - 1)
            @pl.when(i + 1 < NB)
            def _():
                x_cp(nxt).wait()
            r0 = pl.multiple_of(i * TM, TM)
            xn = xn_v[pl.ds(r0, TM), :]
            k = jnp.dot(xn, wk_v[...], preferred_element_type=f32)
            pk = _phi(k)
            z_v[...] += jnp.sum(pk.reshape(TM // 8, 8, D), axis=0)
            pkb = pk.astype(bf16)
            v = jnp.dot(xn, wv_v[...], preferred_element_type=f32).astype(bf16)
            for g in range(G):
                sl = slice(g * 128, (g + 1) * 128)
                kv_v[sl, :] += lax.dot_general(pkb[:, sl], v[:, sl], (((0,), (0,)), ((), ())),
                                               preferred_element_type=f32)
            ln_block(nxt)
            return carry
        lax.fori_loop(0, NB, pass1, 0)

        r_all = r_v[...]
        rmax = jnp.max(r_all)
        rows_i = lax.broadcasted_iota(jnp.int32, (S, 1), 0)
        idx = jnp.min(jnp.where(r_all == rmax, rows_i, S))
        idx = jnp.minimum(idx, S - 1)
        idx16 = pl.multiple_of((idx // 16) * 16, 16)
        xs = xn_v[pl.ds(idx16, 16), :]

        ri = lax.broadcasted_iota(jnp.int32, (128, 128), 0) // DH
        ci = lax.broadcasted_iota(jnp.int32, (128, 128), 1) // DH
        same = ri == ci
        z = jnp.sum(z_v[...], axis=0, keepdims=True)
        wq_cp.wait()
        wo_cp.wait()
        for g in range(G):
            sl = slice(g * 128, (g + 1) * 128)
            kvb = jnp.where(same, kv_v[sl, :], 0.0).astype(bf16)
            m_v[sl, :] = jnp.dot(kvb, wo_v[sl, :], preferred_element_type=f32).astype(bf16)
            zt_v[sl, :] = jnp.where(same, jnp.broadcast_to(z[:, sl], (128, 128)), 0.0).astype(bf16)

        def q_block(i):
            r0 = pl.multiple_of(i * TM, TM) if not isinstance(i, int) else i * TM
            xn = xn_v[pl.ds(r0, TM), :]
            q = jnp.dot(xn, wq_v[...], preferred_element_type=f32)
            pq = _phi(q)
            pqb = pq.astype(bf16)
            outs = []
            for g in range(G):
                sl = slice(g * 128, (g + 1) * 128)
                den = lax.dot_general(pqb[:, sl], zt_v[sl, :], (((1,), (1,)), ((), ())),
                                      preferred_element_type=f32) + 1e-6
                outs.append((pq[:, sl] / den).astype(bf16))
            op_v[pl.ds(r0, TM), :] = jnp.concatenate(outs, axis=1)

        q_block(0)
        y_v[...] = jnp.zeros_like(y_v)

        def pass2(i, carry):
            @pl.when(i > 0)
            def _():
                o_cp(jnp.maximum(i - 1, 0)).start()
            g_cp(i).wait()
            u_cp(i).wait()
            d_cp(i).wait()
            c0 = pl.multiple_of(i * CH, 128)
            gt = jnp.dot(xs, wg_v[:, pl.ds(c0, CH)], preferred_element_type=f32)
            ut = jnp.dot(xs, wu_v[:, pl.ds(c0, CH)], preferred_element_type=f32)
            h = (gt * jax.nn.sigmoid(gt) * ut).astype(bf16)
            y_v[...] += jnp.dot(h, wd_v[pl.ds(c0, CH), :], preferred_element_type=f32)

            r0 = pl.multiple_of(i * TM, TM)
            rows = pl.ds(r0, TM)
            acc = jnp.dot(op_v[rows, :], m_v[...], preferred_element_type=f32)
            out_v[rows, :] = (acc + x_v[rows, :].astype(f32) + xn_v[rows, :].astype(f32)).astype(bf16)
            q_block(jnp.minimum(i + 1, NB - 1))
            return carry
        lax.fori_loop(0, NB, pass2, 0)

        for i in range(NB - 1):
            o_cp(i).wait()
        gate = jax.nn.sigmoid(jnp.full((1, 1), rmax, f32))
        slab = pl.ds(idx16, 16)
        rr = lax.broadcasted_iota(jnp.int32, (16, D), 0)
        cur = out_v[slab, :]
        upd = (cur.astype(f32) + y_v[...] * gate).astype(bf16)
        out_v[slab, :] = jnp.where(rr == idx - idx16, upd, cur)
        o_cp(NB - 1).start()
        p_cp = pltpu.make_async_copy(out_v.at[slab, :], out_hbm.at[slab, :], p_sem.at[0])
        sel_early = idx < (NB - 1) * TM
        @pl.when(sel_early)
        def _():
            p_cp.start()
        o_cp(NB - 1).wait()
        @pl.when(sel_early)
        def _():
            p_cp.wait()

    any_spec = pl.BlockSpec(memory_space=pl.ANY)
    scratch = [
        pltpu.VMEM((S, D), bf16),
        pltpu.VMEM((S, D), bf16),
        pltpu.VMEM((D, D), bf16),
        pltpu.VMEM((D, D), bf16),
        pltpu.VMEM((D, D), bf16),
        pltpu.VMEM((D, D), bf16),
        pltpu.VMEM((D, D), bf16),
        pltpu.VMEM((D,), bf16),
        pltpu.VMEM((D, F), bf16),
        pltpu.VMEM((D, F), bf16),
        pltpu.VMEM((F, D), bf16),
        pltpu.VMEM((D, 128), f32),
        pltpu.VMEM((8, D), f32),
        pltpu.VMEM((D, 128), bf16),
        pltpu.VMEM((S, 1), f32),
        pltpu.VMEM((S, D), bf16),
        pltpu.VMEM((S, D), bf16),
        pltpu.VMEM((16, D), f32),
        pltpu.SemaphoreType.DMA((NB,)),
        pltpu.SemaphoreType.DMA((5,)),
        pltpu.SemaphoreType.DMA((NB,)),
        pltpu.SemaphoreType.DMA((NB,)),
        pltpu.SemaphoreType.DMA((NB,)),
        pltpu.SemaphoreType.DMA((NB,)),
        pltpu.SemaphoreType.DMA((1,)),
    ]

    def run(A_x, A_wqkv, A_wo, B_x, B_w_r, B_w_gate, B_w_up, B_w_down):
        out = pl.pallas_call(
            kernel,
            out_shape=jax.ShapeDtypeStruct((S, D), bf16),
            in_specs=[any_spec] * 7,
            out_specs=any_spec,
            scratch_shapes=scratch,
            compiler_params=pltpu.CompilerParams(vmem_limit_bytes=100 * 2**20),
        )(A_x.reshape(S, D), A_wqkv, A_wo, B_w_r, B_w_gate, B_w_up, B_w_down)
        return out.reshape(1, S, D)
    return jax.jit(run)


_run = make_kernel()


@jax.jit
def pallas_parallel_sum__linear_attn_block__moe_arch_mod__prompt_kernel(
    A_x: jax.Array,
    A_wqkv: jax.Array,
    A_wo: jax.Array,
    B_x: jax.Array,
    B_w_r: jax.Array,
    B_w_gate: jax.Array,
    B_w_up: jax.Array,
    B_w_down: jax.Array,
):
    return _run(A_x, A_wqkv, A_wo, B_x, B_w_r, B_w_gate, B_w_up, B_w_down)
```

```python
import functools
import numpy as np
import jax
import jax.numpy as jnp
from jax import lax
from jax.experimental import pallas as pl
from jax.experimental.pallas import tpu as pltpu

S, D, H, DH, F = 2048, 1024, 32, 32, 3584
G = D // 128
f32, bf16, u32 = jnp.float32, jnp.bfloat16, jnp.uint32
EPS_B = 1.00135803e-05
FLAGS = {"XLA_TPU_EVENLY_DISTRIBUTE_CRITICAL_NODES": True}


def _rb(x):
    return x.astype(bf16).astype(f32)


def _phi(t):
    return jnp.where(t > 0, t + 1.0, jnp.exp(t)) + 1e-6


def _dot(a, b):
    return jnp.dot(a, b, preferred_element_type=f32)


def _pack(x):
    return pltpu.bitcast(x.astype(bf16), u32)


def _unpack(w):
    return pltpu.bitcast(w, bf16)


def _bits(x):
    return pltpu.bitcast(x, u32)


def _tiles(x):
    return [x[r:r + 8, c:c + 128] for r in range(0, x.shape[0], 8) for c in range(0, x.shape[1], 128)]


def _or_all(ts):
    return functools.reduce(jnp.bitwise_or, ts)


class _Null:
    def __enter__(self):
        return self
    def __exit__(self, *a):
        return False


def make_kernel(TM=512, CR=32, CH=512, X0=2, KB=16, SL=64, flags=None, scopes=False, moe="vpu",
                lnpos=0.0, lag=0.0, span=0.95, split=True, anchor=True, fuse=False,
                WSL=((0, 1), (1, 1), (2, 2), (4, 2), (6, 2)), X1AFTER=2, X1WAIT=4, late=False):
    NB = S // TM
    NC = F // CH
    NLN = TM // CR
    XR = TM // X0
    W = 256

    def scope(name):
        return jax.named_scope(name) if scopes else _Null()

    def kernel(x_hbm, wqkv_hbm, wo_hbm, wr_hbm, wg_hbm, wu_hbm, wd_hbm, out_hbm,
               x_v, xn32, wq_v, wk_v, wv_v, wo_v, m32, op32, wr_v, wg_v, wu_v, wd_v, out_v, xb_v, hb_v,
               x0_sem, x_sem, k_sem, v_sem, w_sem, o_sem):
        NW = D // W
        def cp(src, dst, sem):
            return pltpu.make_async_copy(src, dst, sem)
        def x0_cp(c):
            return cp(x_hbm.at[pl.ds(c * XR, XR), :], x_v.at[pl.ds(c * XR, XR), :], x0_sem.at[c])
        def x_cp(i):
            return cp(x_hbm.at[pl.ds(i * TM, TM), :], x_v.at[pl.ds(i * TM, TM), :], x_sem.at[i])
        def x1_cp(h):
            r0 = TM + h * (TM // 2)
            return cp(x_hbm.at[pl.ds(r0, TM // 2), :], x_v.at[pl.ds(r0, TM // 2), :], x_sem.at[h])
        def wk_cp(j):
            g0, ng = WSL[j]
            return cp(wqkv_hbm.at[:, pl.ds(D + g0 * 128, ng * 128)], wk_v.at[:, pl.ds(g0 * 128, ng * 128)], k_sem.at[j])
        def wv_cp(j):
            g0, ng = WSL[j]
            return cp(wqkv_hbm.at[:, pl.ds(2 * D + g0 * 128, ng * 128)], wv_v.at[:, pl.ds(g0 * 128, ng * 128)], v_sem.at[j])
        wq_cp = cp(wqkv_hbm.at[:, pl.ds(0, D)], wq_v, w_sem.at[0])
        wo_cp = cp(wo_hbm, wo_v, w_sem.at[1])
        wr_cp = cp(wr_hbm, wr_v, w_sem.at[2])
        wg_cp = cp(wg_hbm, wg_v, w_sem.at[3])
        wu_cp = cp(wu_hbm, wu_v, w_sem.at[4])
        wd_cp = cp(wd_hbm, wd_v, w_sem.at[5])
        def o_cp(i):
            return cp(out_v.at[pl.ds(i * TM, TM), :], out_hbm.at[pl.ds(i * TM, TM), :], o_sem.at[i])
        def ol_cp(n):
            r0 = (NB - 1) * TM
            return cp(out_v.at[pl.ds(r0, TM), pl.ds(n * W, W)],
                      out_hbm.at[pl.ds(r0, TM), pl.ds(n * W, W)], o_sem.at[NB - 1 + n])

        x0s = [x0_cp(c) for c in range(X0)]
        wks = [wk_cp(j) for j in range(len(WSL))]
        wvs = [wv_cp(j) for j in range(len(WSL))]
        xs_ = {i: x_cp(i) for i in range(2, NB)}
        x1s = [x1_cp(0), x1_cp(1)]
        if X0 == 4:
            queue = {
                "begin": [wr_cp, x0s[0], x0s[1]],
                ("x0", 0): [x0s[2], x0s[3]],
                ("x0", 1): [wks[0], wvs[0]],
                ("x0", 2): [wks[1], wvs[1]],
                ("x0", 3): [wks[2], wvs[2]],
            }
        else:
            queue = {
                "begin": [wr_cp, x0s[0], x0s[1], wks[0], wvs[0]],
                ("x0", 0): [wks[1], wvs[1]],
                ("x0", 1): [wks[2], wvs[2]],
            }
        queue.update({
            ("w", 0): [x1s[0]],
            ("w", 1): [wks[3], wvs[3]],
            ("w", 2): [wks[4], wvs[4], x1s[1]],
            ("w", 3): [xs_[2]],
            ("w", 4): [xs_[3]],
        })
        for c_ in (wg_cp, wu_cp, wq_cp, wo_cp, wd_cp):
            c_.start(priority=1)
        def kick(key):
            for c_ in queue.pop(key, ()):
                c_.start()
        kick("begin")

        st = dict(best=None, bidx=None)

        def never(tok):
            return pltpu.bitcast(tok, f32) > st["big"]

        def mm(lhs_w, rhs, side=()):
            if not side or not split:
                res = _dot(_unpack(lhs_w), rhs)
                for pos, thunk in side:
                    r = min(int(pos * (TM // 8)), TM // 8 - 1)
                    thunk(res[r * 8:(r + 1) * 8, :] if anchor else None)
                return res
            hd = D // 2
            res = None
            for h in range(2):
                part = _dot(_unpack(lhs_w[:, h * hd:(h + 1) * hd]), rhs[h * hd:(h + 1) * hd, :])
                for pos, thunk in side:
                    if (pos >= 0.5) == (h == 1):
                        r = min(int((pos * 2 - h) * (TM // 8)), TM // 8 - 1)
                        thunk(part[r * 8:(r + 1) * 8, :] if anchor else None)
                res = part if res is None else res + part
            return res

        def gated(x, tok):
            if tok is None:
                return x
            m = tok > st["big"]
            m = jnp.concatenate([m] * (x.shape[1] // 128), axis=1) if x.shape[1] > 128 else m[:, :x.shape[1]]
            m = jnp.concatenate([m] * (x.shape[0] // 8), axis=0) if x.shape[0] > 8 else m
            return jnp.where(m, 0.0, x)

        def spread(q, k, lo=0.0, hi=1.0):
            items = [q.pop(0) for _ in range(min(k, len(q)))]
            return [(lo + (hi - lo) * j / len(items), f) for j, f in enumerate(items)]

        def ln_piece(i, c, tok=None):
            r0 = i * TM + c * CR
            xf = x_v[pl.ds(r0, CR), :].astype(f32)
            mean = gated(jnp.sum(xf, axis=1, keepdims=True), tok) * (1.0 / D)
            mb = _rb(mean)
            d = xf - mb
            dm = mean - mb
            var = jnp.sum(d * d, axis=1, keepdims=True) * (1.0 / D) - dm * dm
            rs = jnp.sum(d * st["wr"], axis=1, keepdims=True)
            inv = 1.0 / _rb(jnp.sqrt(_rb(_rb(var) + EPS_B)))
            r = _rb(rs * inv)
            packed = _pack(d * inv)
            xn32[pl.ds(r0 // 2, CR // 2), :] = packed
            ridx = lax.broadcasted_iota(jnp.int32, (CR, 1), 0) + r0
            if st["best"] is None:
                st["best"], st["bidx"] = r, ridx
            else:
                take = r > st["best"]
                st["best"] = jnp.where(take, r, st["best"])
                st["bidx"] = jnp.where(take, ridx, st["bidx"])

        def xw(i):
            return xn32[pl.ds(i * TM // 2, TM // 2), :]

        for c0 in range(X0):
            with scope(f"wait_x0_{c0}"):
                if c0 == 0:
                    wr_cp.wait()
                x0s[c0].wait()
            kick(("x0", c0))
            if c0 == 0:
                st["wr"] = wr_v[...].astype(f32).reshape(1, D)
                wbits = pltpu.bitcast(jnp.broadcast_to(st["wr"][:, 0:128], (8, 128)), jnp.int32)
                st["big"] = pltpu.bitcast(((wbits | 1) & 1) * 0x7F800000, f32)
            for c in range(c0 * NLN // X0, (c0 + 1) * NLN // X0):
                ln_piece(0, c)

        pkb, vb = {}, {}
        kv = [None] * G
        zacc = [None] * G

        def K(i, g, side=()):
            pk = _phi(mm(xw(i), wk_v[:, g * 128:(g + 1) * 128], side))
            zp = jnp.sum(pk.reshape(TM // 8, 8, 128), axis=0)
            zacc[g] = zp if zacc[g] is None else zacc[g] + zp
            pkb[i, g] = pk.astype(bf16)

        def V(i, g, side=()):
            vb[i, g] = mm(xw(i), wv_v[:, g * 128:(g + 1) * 128], side).astype(bf16)

        def KV(i, g):
            p = lax.dot_general(pkb.pop((i, g)), vb.pop((i, g)), (((0,), (0,)), ((), ())),
                                preferred_element_type=f32)
            kv[g] = p if kv[g] is None else kv[g] + p

        ys = dict(yv=None)

        def col_bcast(dst, k0, row):
            for t in range(row.shape[1] // 128):
                blk = jnp.broadcast_to(row[:, t * 128:(t + 1) * 128], (128, 128))
                dst[pl.ds(k0 + t * 128, 128), :] = blk.T

        def mv_step(accs, b_ref, k0, nk, w_refs, c0, nc, tok=None):
            for kb in range(nk // KB):
                rows = pl.ds(k0 + kb * KB, KB)
                bb = gated(b_ref[rows, :], tok)
                bt = jnp.concatenate([bb] * (nc // 128), axis=1)
                for j, w_ref in enumerate(w_refs):
                    p = w_ref[rows, pl.ds(c0, nc)].astype(f32) * bt
                    p = jnp.sum(p.reshape(KB // 8, 8, nc), axis=0)
                    accs[j] = p if accs[j] is None else accs[j] + p

        def gu_slices(c):
            accs = [None, None]
            out = [functools.partial(mv_step, accs, xb_v, k0, SL, [wg_v, wu_v], c * CH, CH)
                   for k0 in range(0, D, SL)]
            def fin(tok=None):
                gt = jnp.sum(accs[0], axis=0, keepdims=True)
                ut = jnp.sum(accs[1], axis=0, keepdims=True)
                h = _rb(gt * jax.nn.sigmoid(gt) * ut)
                col_bcast(hb_v, c * CH, h)
            return out + [fin]

        def dn_slices(c):
            def step(k0, tok=None):
                accs = [ys["yv"]]
                mv_step(accs, hb_v, k0, SL // 2, [wd_v], 0, D, tok)
                ys["yv"] = accs[0]
            return [functools.partial(step, k0) for k0 in range(c * CH, (c + 1) * CH, SL // 2)]

        moe1 = [f for c in range(NC) for f in gu_slices(c)]
        moe2 = [f for c in range(NC) for f in dn_slices(c)]
        n1 = -(-len(moe1) // 16)
        n2 = -(-len(moe2) // 22)

        rt = {}
        def route():
            best, bidx = st["best"], st["bidx"]
            rmax = jnp.max(best)
            idx = jnp.min(jnp.where(best == rmax, bidx, S))
            idx = jnp.minimum(idx, S - 1)
            idx16 = pl.multiple_of((idx // 16) * 16, 16)
            rt.update(rmax=rmax, idx=idx, idx16=idx16)
            slab = _unpack(xn32[pl.ds(pl.multiple_of(idx16 // 2, 8), 8), :])
            rr16 = lax.broadcasted_iota(jnp.int32, (16, D), 0)
            xrow = jnp.sum(jnp.where(rr16 == idx - idx16, slab.astype(f32), 0.0), axis=0, keepdims=True)
            col_bcast(xb_v, 0, xrow)

        pend = []
        for i in range(NB):
            lastb = i == NB - 1
            lnq = [] if lastb else [functools.partial(ln_piece, i + 1, c) for c in range(NLN)]
            for g in range(G):
                n = g // 2
                if i == 0:
                    for j, (g0, ng) in enumerate(WSL):
                        if g == g0:
                            with scope(f"wait_w{j}"):
                                wk_cp(j).wait()
                                wv_cp(j).wait()
                                if g == 4:
                                    x1s[0].wait()
                                if g == 6:
                                    x1s[1].wait()
                            kick(("w", j))
                if i == 1 and g == 2:
                    with scope("wait_x"):
                        for j in range(2, NB):
                            xs_[j].wait()
                if lastb and g == 0:
                    with scope("wait_gu"):
                        wg_cp.wait()
                        wu_cp.wait()
                    route()
                for MAT in (K, V):
                    if lastb:
                        side = spread(moe1, n1, 0.0, span)
                    elif i == 0:
                        side = spread(lnq, 2 * NLN // 16, lnpos, span) if g >= 4 else []
                    elif i == 1:
                        left = 2 * (G - g) - (MAT is V)
                        side = spread(lnq, -(-len(lnq) // left), lnpos, span) if g >= 2 else []
                    else:
                        side = spread(lnq, -(-NLN // 16), lnpos, span)
                    MAT(i, g, side)
                if len(pend) >= 1:
                    KV(*pend.pop(0))
                pend.append((i, g))
            assert not lnq
        for f in moe1:
            f(None)
        del moe1[:]

        idx, idx16, rmax = rt["idx"], rt["idx16"], rt["rmax"]
        ri = lax.broadcasted_iota(jnp.int32, (128, 128), 0) // DH
        ci = lax.broadcasted_iota(jnp.int32, (128, 128), 1) // DH
        same = ri == ci

        zt = {}
        def Mp(g):
            kvb = jnp.where(same, kv[g], 0.0).astype(bf16)
            m32[g * 64:(g + 1) * 64, :] = _pack(_dot(kvb, wo_v[g * 128:(g + 1) * 128, :]))

        def ZT(g):
            z = jnp.sum(zacc[g], axis=0, keepdims=True)
            zt[g] = jnp.where(same, jnp.broadcast_to(z, (128, 128)), 0.0).astype(bf16)

        def dside():
            return spread(moe2, n2, 0.0, span)

        pq = {}
        def Q(i, g):
            p = _phi(mm(xw(i), wq_v[:, g * 128:(g + 1) * 128], dside()))
            pq[i, g] = (p, p.astype(bf16))

        def DEN(i, g):
            p, pb = pq.pop((i, g))
            den = lax.dot_general(pb, zt[g], (((1,), (1,)), ((), ())),
                                  preferred_element_type=f32) + 1e-6
            rc = pl.reciprocal(den, approx=True)
            rc = rc * (2.0 - den * rc)
            op32[pl.ds(i * TM // 2, TM // 2), g * 128:(g + 1) * 128] = _pack(p * rc)

        def OUT(i, g):
            cols = slice(g * 128, (g + 1) * 128)
            acc = mm(op32[pl.ds(i * TM // 2, TM // 2), :], _unpack(m32[:, cols]), dside())
            res = (x_v[pl.ds(i * TM, TM), cols].astype(f32)
                   + _unpack(xn32[pl.ds(i * TM // 2, TM // 2), cols]).astype(f32))
            out_v[pl.ds(i * TM, TM), cols] = (acc + res).astype(bf16)

        with scope("wait_qod"):
            wq_cp.wait()
            wo_cp.wait()
            wd_cp.wait()
        for g in range(G):
            ZT(g)
        Q(0, 0)
        KV(*pend.pop(0))
        assert not pend
        Q(0, 1)
        Mp(0); Mp(1)
        Q(0, 2)
        DEN(0, 0)
        Mp(2); Mp(3)
        Q(0, 3)
        DEN(0, 1)
        Mp(4); Mp(5)
        Q(0, 4)
        DEN(0, 2)
        Mp(6); Mp(7)
        Q(0, 5)
        DEN(0, 3)
        Q(0, 6)
        DEN(0, 4)
        Q(0, 7)
        DEN(0, 5)

        gate = jax.nn.sigmoid(jnp.full((1, 1), rmax, f32))
        rr = lax.broadcasted_iota(jnp.int32, (16, D), 0)

        def patch(i, cols=slice(None)):
            slab = pl.multiple_of(jnp.clip(idx16, i * TM, (i + 1) * TM - 16), 16)
            cur = out_v[pl.ds(slab, 16), cols]
            upd = (cur.astype(f32) + ys["yg"][:, cols]).astype(bf16)
            out_v[pl.ds(slab, 16), cols] = jnp.where(rr[:, cols] + slab == idx, upd, cur)

        for i in range(NB):
            if i + 1 < NB:
                Q(i + 1, 0)
                if i == 0:
                    DEN(0, 6)
                Q(i + 1, 1)
                if i == 0:
                    DEN(0, 7)
                Q(i + 1, 2)
                DEN(i + 1, 0)
                for g in range(G):
                    OUT(i, g)
                    if g + 3 < G:
                        Q(i + 1, g + 3)
                    DEN(i + 1, g + 1) if g + 1 < G else None
                if i == 0:
                    for f in moe2:
                        f(None)
                    del moe2[:]
                    ys["yg"] = jnp.broadcast_to(jnp.sum(ys["yv"], axis=0, keepdims=True), (16, D)) * gate
                patch(i)
                o_cp(i).start()
            else:
                for n in range(NW):
                    OUT(i, 2 * n)
                    OUT(i, 2 * n + 1)
                    patch(i, slice(n * W, (n + 1) * W))
                    ol_cp(n).start()
        with scope("wait_out"):
            for i in range(NB - 1):
                o_cp(i).wait()
            for n in range(NW):
                ol_cp(n).wait()

    any_spec = pl.BlockSpec(memory_space=pl.ANY)
    scratch = [
        pltpu.VMEM((S, D), bf16),
        pltpu.VMEM((S // 2, D), u32),
        pltpu.VMEM((D, D), bf16),
        pltpu.VMEM((D, D), bf16),
        pltpu.VMEM((D, D), bf16),
        pltpu.VMEM((D, D), bf16),
        pltpu.VMEM((D // 2, D), u32),
        pltpu.VMEM((S // 2, D), u32),
        pltpu.VMEM((D,), bf16),
        pltpu.VMEM((D, F), bf16),
        pltpu.VMEM((D, F), bf16),
        pltpu.VMEM((F, D), bf16),
        pltpu.VMEM((S, D), bf16),
        pltpu.VMEM((D, 128), f32),
        pltpu.VMEM((F, 128), f32),
        pltpu.SemaphoreType.DMA((X0,)),
        pltpu.SemaphoreType.DMA((S // TM,)),
        pltpu.SemaphoreType.DMA((len(WSL),)),
        pltpu.SemaphoreType.DMA((len(WSL),)),
        pltpu.SemaphoreType.DMA((6,)),
        pltpu.SemaphoreType.DMA((S // TM - 1 + 4,)),
    ]

    def run(A_x, A_wqkv, A_wo, B_x, B_w_r, B_w_gate, B_w_up, B_w_down):
        out = pl.pallas_call(
            kernel,
            out_shape=jax.ShapeDtypeStruct((S, D), bf16),
            in_specs=[any_spec] * 7,
            out_specs=any_spec,
            scratch_shapes=scratch,
            compiler_params=pltpu.CompilerParams(vmem_limit_bytes=120 * 2**20, flags=flags, fuse_transposed_lhs_in_matmul=fuse),
        )(A_x.reshape(S, D), A_wqkv, A_wo, B_w_r, B_w_gate, B_w_up, B_w_down)
        return out.reshape(1, S, D)
    return jax.jit(run)


_run = make_kernel(SL=32,CR=32,X0=2)


@jax.jit
def pallas_parallel_sum__linear_attn_block__moe_arch_mod__prompt_kernel(
    A_x: jax.Array,
    A_wqkv: jax.Array,
    A_wo: jax.Array,
    B_x: jax.Array,
    B_w_r: jax.Array,
    B_w_gate: jax.Array,
    B_w_up: jax.Array,
    B_w_down: jax.Array,
):
    return _run(A_x, A_wqkv, A_wo, B_x, B_w_r, B_w_gate, B_w_up, B_w_down)
```

```python
import functools
import numpy as np
import jax
import jax.numpy as jnp
from jax import lax
from jax.experimental import pallas as pl
from jax.experimental.pallas import tpu as pltpu

S, D, H, DH, F = 2048, 1024, 32, 32, 3584
G = D // 128
f32, bf16, u32 = jnp.float32, jnp.bfloat16, jnp.uint32
EPS_B = 1.00135803e-05
FLAGS = {"XLA_TPU_EVENLY_DISTRIBUTE_CRITICAL_NODES": True}


def _rb(x):
    return x.astype(bf16).astype(f32)


def _phi(t):
    return jnp.where(t > 0, t + 1.0, jnp.exp(t)) + 1e-6


def _dot(a, b):
    return jnp.dot(a, b, preferred_element_type=f32)


def _pack(x):
    return pltpu.bitcast(x.astype(bf16), u32)


def _unpack(w):
    return pltpu.bitcast(w, bf16)


def _bits(x):
    return pltpu.bitcast(x, u32)


def _tiles(x):
    return [x[r:r + 8, c:c + 128] for r in range(0, x.shape[0], 8) for c in range(0, x.shape[1], 128)]


def _or_all(ts):
    return functools.reduce(jnp.bitwise_or, ts)


class _Null:
    def __enter__(self):
        return self
    def __exit__(self, *a):
        return False


def make_kernel(TM=512, CR=32, CH=512, X0=2, KB=16, SL=64, flags=None, scopes=False, moe="vpu",
                lnpos=0.0, lag=0.0, span=0.95, split=True, anchor=True, fuse=False,
                WSL=((0, 1), (1, 1), (2, 2), (4, 2), (6, 2)), NSLOT2=22, kvx=(0, 1, 2), nodma=False, endanch=True, ENDROW=1, ENDK=4):
    NB = S // TM
    NC = F // CH
    NLN = TM // CR
    XR = TM // X0
    W = 256

    def scope(name):
        return jax.named_scope(name) if scopes else _Null()

    def kernel(x_hbm, wqkv_hbm, wo_hbm, wr_hbm, wg_hbm, wu_hbm, wd_hbm, out_hbm,
               x_v, xn32, wq_v, wk_v, wv_v, wo_v, m32, op32, wr_v, wg_v, wu_v, wd_v, out_v, xb_v, hb_v,
               wqt32, zc_v,
               x0_sem, x_sem, k_sem, v_sem, w_sem, o_sem):
        NW = D // W
        def cp(src, dst, sem):
            return pltpu.make_async_copy(src, dst, sem)
        def x0_cp(c):
            return cp(x_hbm.at[pl.ds(c * XR, XR), :], x_v.at[pl.ds(c * XR, XR), :], x0_sem.at[c])
        def x_cp(i):
            return cp(x_hbm.at[pl.ds(i * TM, TM), :], x_v.at[pl.ds(i * TM, TM), :], x_sem.at[i])
        def x1_cp(h):
            r0 = TM + h * (TM // 2)
            return cp(x_hbm.at[pl.ds(r0, TM // 2), :], x_v.at[pl.ds(r0, TM // 2), :], x_sem.at[h])
        def wk_cp(j):
            g0, ng = WSL[j]
            return cp(wqkv_hbm.at[:, pl.ds(D + g0 * 128, ng * 128)], wk_v.at[:, pl.ds(g0 * 128, ng * 128)], k_sem.at[j])
        def wv_cp(j):
            g0, ng = WSL[j]
            return cp(wqkv_hbm.at[:, pl.ds(2 * D + g0 * 128, ng * 128)], wv_v.at[:, pl.ds(g0 * 128, ng * 128)], v_sem.at[j])
        wq_cp = cp(wqkv_hbm.at[:, pl.ds(0, D)], wq_v, w_sem.at[0])
        wo_cp = cp(wo_hbm, wo_v, w_sem.at[1])
        wr_cp = cp(wr_hbm, wr_v, w_sem.at[2])
        wg_cp = cp(wg_hbm, wg_v, w_sem.at[3])
        wu_cp = cp(wu_hbm, wu_v, w_sem.at[4])
        wd_cp = cp(wd_hbm, wd_v, w_sem.at[5])
        def o_cp(i):
            return cp(out_v.at[pl.ds(i * TM, TM), :], out_hbm.at[pl.ds(i * TM, TM), :], o_sem.at[i])
        def ol_cp(n):
            r0 = (NB - 1) * TM
            return cp(out_v.at[pl.ds(r0, TM), pl.ds(n * W, W)],
                      out_hbm.at[pl.ds(r0, TM), pl.ds(n * W, W)], o_sem.at[NB - 1 + n])

        x0s = [x0_cp(c) for c in range(X0)]
        wks = [wk_cp(j) for j in range(len(WSL))]
        wvs = [wv_cp(j) for j in range(len(WSL))]
        xs_ = {i: x_cp(i) for i in range(2, NB)}
        x1s = [x1_cp(0), x1_cp(1)]
        if X0 == 4:
            queue = {
                "begin": [wr_cp, x0s[0], x0s[1]],
                ("x0", 0): [x0s[2], x0s[3]],
                ("x0", 1): [wks[0], wvs[0]],
                ("x0", 2): [wks[1], wvs[1]],
                ("x0", 3): [wks[2], wvs[2]],
            }
        else:
            queue = {
                "begin": [wr_cp, x0s[0], x0s[1], wks[0], wvs[0]],
                ("x0", 0): [wks[1], wvs[1]],
                ("x0", 1): [wks[2], wvs[2]],
            }
        queue.update({
            ("w", 0): [x1s[0]],
            ("w", 1): [wks[3], wvs[3]],
            ("w", 2): [wks[4], wvs[4], x1s[1]],
            ("w", 3): [xs_[2]],
            ("w", 4): [xs_[3]],
        })
        queue["begin_lo"] = [wq_cp]
        if nodma:
            tiny = lambda j: cp(wg_hbm.at[pl.ds(0, 16), pl.ds(0, 128)], wg_v.at[pl.ds(16 * j, 16), pl.ds(0, 128)], w_sem.at[j])
            wg_cp, wu_cp, wd_cp = tiny(3), tiny(4), tiny(5)
        queue[("x0", 0, "lo")] = [wg_cp]
        queue[("w", 0, "lo")] = [wu_cp]
        queue[("w", 1, "lo")] = [wo_cp]
        queue[("w", 2, "lo")] = [wd_cp]
        def kick(key):
            for c_ in queue.pop(key, ()):
                c_.start()
            lo = "begin_lo" if key == "begin" else key + ("lo",)
            for c_ in queue.pop(lo, ()):
                c_.start(priority=1)
        kick("begin")

        st = dict(best=None, bidx=None, endq=[])

        def never(tok):
            return pltpu.bitcast(tok, f32) > st["big"]

        def mm(lhs_w, rhs, side=(), nt=False):
            dn = (((1,), (1,)), ((), ())) if nt else (((1,), (0,)), ((), ()))
            R = lhs_w.shape[0] // 4
            hd = D // 2
            if st["endq"] and not nt:
                tok = _or_all(st["endq"])
                del st["endq"][:]
                rg, kk = lhs_w.shape[0] // 8 - ENDROW, ENDK
                m = pltpu.bitcast(tok, f32) > st["big"]
                blk = lhs_w[rg * 8:(rg + 1) * 8, :]
                tl = blk[:, kk * 128:(kk + 1) * 128]
                tl = jnp.where(m, jnp.zeros_like(tl), tl)
                blk = jnp.concatenate([blk[:, :kk * 128], tl, blk[:, (kk + 1) * 128:]], axis=1) if kk < G - 1 else \
                    jnp.concatenate([blk[:, :kk * 128], tl], axis=1)
                parts = [lhs_w[:rg * 8], blk] + ([lhs_w[(rg + 1) * 8:]] if (rg + 1) * 8 < lhs_w.shape[0] else [])
                lhs_w = jnp.concatenate(parts, axis=0)
            if not side:
                return lax.dot_general(_unpack(lhs_w), rhs, dn, preferred_element_type=f32)
            res = None
            newq = []
            for h in range(2):
                ks = slice(h * hd, (h + 1) * hd)
                part = lax.dot_general(_unpack(lhs_w[:, ks]), rhs[:, ks] if nt else rhs[ks, :], dn,
                                       preferred_element_type=f32)
                for pos, thunk in side:
                    if (pos >= 0.5) == (h == 1):
                        r = min(int((pos * 2 - h) * R), R - 1)
                        t_ = thunk(part[r * 8:(r + 1) * 8, 0:128] if anchor else None)
                        if t_ is not None:
                            newq.append(t_)
                res = part if res is None else res + part
            st["endq"].extend(newq)
            return res

        def gated(x, tok):
            if tok is None:
                return x
            m = tok > st["big"]
            m = jnp.concatenate([m] * (x.shape[1] // 128), axis=1) if x.shape[1] > 128 else m[:, :x.shape[1]]
            m = jnp.concatenate([m] * (x.shape[0] // 8), axis=0) if x.shape[0] > 8 else m
            return jnp.where(m, 0.0, x)

        def spread(q, k, lo=0.0, hi=1.0):
            items = [q.pop(0) for _ in range(min(k, len(q)))]
            return [(lo + (hi - lo) * j / len(items), f) for j, f in enumerate(items)]

        def ln_piece(i, c, tok=None):
            r0 = i * TM + c * CR
            xf = x_v[pl.ds(r0, CR), :].astype(f32)
            mean = gated(jnp.sum(xf, axis=1, keepdims=True), tok) * (1.0 / D)
            mb = _rb(mean)
            d = xf - mb
            dm = mean - mb
            var = jnp.sum(d * d, axis=1, keepdims=True) * (1.0 / D) - dm * dm
            rs = jnp.sum(d * st["wr"], axis=1, keepdims=True)
            inv = 1.0 / _rb(jnp.sqrt(_rb(_rb(var) + EPS_B)))
            r = _rb(rs * inv)
            packed = _pack(d * inv)
            xn32[pl.ds(r0 // 2, CR // 2), :] = packed
            ridx = lax.broadcasted_iota(jnp.int32, (CR, 1), 0) + r0
            if st["best"] is None:
                st["best"], st["bidx"] = r, ridx
            else:
                take = r > st["best"]
                st["best"] = jnp.where(take, r, st["best"])
                st["bidx"] = jnp.where(take, ridx, st["bidx"])
            if endanch and tok is not None:
                return _or_all(_tiles(packed))

        def xw(i):
            return xn32[pl.ds(i * TM // 2, TM // 2), :]

        for c0 in range(X0):
            with scope(f"wait_x0_{c0}"):
                if c0 == 0:
                    wr_cp.wait()
                x0s[c0].wait()
            kick(("x0", c0))
            if c0 == 0:
                st["wr"] = wr_v[...].astype(f32).reshape(1, D)
                wbits = pltpu.bitcast(jnp.broadcast_to(st["wr"][:, 0:128], (8, 128)), jnp.int32)
                one = (wbits | 1) & 1
                st["big"] = pltpu.bitcast(one * 0x7F800000, f32)
                st["zero"] = pltpu.bitcast(jnp.concatenate([(one - 1)] * 8, axis=0), u32)
            for c in range(c0 * NLN // X0, (c0 + 1) * NLN // X0):
                ln_piece(0, c)

        pkb, vb = {}, {}
        kv = [None] * G
        zacc = [None] * G

        def K(i, g, side=()):
            pk = _phi(mm(xw(i), wk_v[:, g * 128:(g + 1) * 128], side))
            zp = jnp.sum(pk.reshape(TM // 8, 8, 128), axis=0)
            zacc[g] = zp if zacc[g] is None else zacc[g] + zp
            pkb[i, g] = pk.astype(bf16)

        def V(i, g, side=()):
            vb[i, g] = mm(xw(i), wv_v[:, g * 128:(g + 1) * 128], side).astype(bf16)

        def KV(i, g):
            if i in kvx:
                kt = pltpu.bitcast(pkb.pop((i, g)).T, u32) | jnp.concatenate([st["zero"][:64]] * (TM // 128), axis=1)
                p = _dot(_unpack(kt), vb.pop((i, g)))
            else:
                p = lax.dot_general(pkb.pop((i, g)), vb.pop((i, g)), (((0,), (0,)), ((), ())),
                                    preferred_element_type=f32)
            kv[g] = p if kv[g] is None else kv[g] + p

        ys = dict(yv=None)

        def col_bcast(dst, k0, row):
            for t in range(row.shape[1] // 128):
                blk = jnp.broadcast_to(row[:, t * 128:(t + 1) * 128], (128, 128))
                dst[pl.ds(k0 + t * 128, 128), :] = blk.T

        def mv_step(accs, b_ref, k0, nk, w_refs, c0, nc, tok=None):
            for kb in range(nk // KB):
                rows = pl.ds(k0 + kb * KB, KB)
                bb = gated(b_ref[rows, :], tok)
                bt = jnp.concatenate([bb] * (nc // 128), axis=1)
                for j, w_ref in enumerate(w_refs):
                    p = w_ref[rows, pl.ds(c0, nc)].astype(f32) * bt
                    p = jnp.sum(p.reshape(KB // 8, 8, nc), axis=0)
                    accs[j] = p if accs[j] is None else accs[j] + p

        def gu_slices(c):
            accs = [None, None]
            out = [functools.partial(mv_step, accs, xb_v, k0, SL, [wg_v, wu_v], c * CH, CH)
                   for k0 in range(0, D, SL)]
            def fin(tok=None):
                gt = jnp.sum(accs[0], axis=0, keepdims=True)
                ut = jnp.sum(accs[1], axis=0, keepdims=True)
                h = _rb(gt * jax.nn.sigmoid(gt) * ut)
                col_bcast(hb_v, c * CH, h)
            return out + [fin]

        def dn_slices(c):
            def step(k0, tok=None):
                accs = [ys["yv"]]
                mv_step(accs, hb_v, k0, SL // 2, [wd_v], 0, D, tok)
                ys["yv"] = accs[0]
            return [functools.partial(step, k0) for k0 in range(c * CH, (c + 1) * CH, SL // 2)]

        def wqt_slab(nt_, tok=None):
            slab = wq_v[:, nt_ * 128:(nt_ + 1) * 128]
            wt = pltpu.bitcast(slab.T, u32)
            wqt32[nt_ * 64:(nt_ + 1) * 64, :] = wt | jnp.concatenate([st["zero"]] * G, axis=1)
        wqtq = [functools.partial(wqt_slab, j) for j in range(G)]

        moe1 = [f for c in range(NC) for f in gu_slices(c)]
        moe2 = [f for c in range(NC) for f in dn_slices(c)]
        n1 = -(-len(moe1) // 16)
        n2 = -(-len(moe2) // NSLOT2)

        rt = {}
        def route():
            best, bidx = st["best"], st["bidx"]
            rmax = jnp.max(best)
            idx = jnp.min(jnp.where(best == rmax, bidx, S))
            idx = jnp.minimum(idx, S - 1)
            idx16 = pl.multiple_of((idx // 16) * 16, 16)
            rt.update(rmax=rmax, idx=idx, idx16=idx16)
            slab = _unpack(xn32[pl.ds(pl.multiple_of(idx16 // 2, 8), 8), :])
            rr16 = lax.broadcasted_iota(jnp.int32, (16, D), 0)
            xrow = jnp.sum(jnp.where(rr16 == idx - idx16, slab.astype(f32), 0.0), axis=0, keepdims=True)
            col_bcast(xb_v, 0, xrow)

        pend = []
        for i in range(NB):
            lastb = i == NB - 1
            lnq = [] if lastb else [functools.partial(ln_piece, i + 1, c) for c in range(NLN)]
            for g in range(G):
                n = g // 2
                if i == 0:
                    for j, (g0, ng) in enumerate(WSL):
                        if g == g0:
                            with scope(f"wait_w{j}"):
                                wk_cp(j).wait()
                                wv_cp(j).wait()
                                if g == 4:
                                    x1s[0].wait()
                                if g == 6:
                                    x1s[1].wait()
                            kick(("w", j))
                if i == 1 and g == 2:
                    with scope("wait_x"):
                        for j in range(2, NB):
                            xs_[j].wait()
                if lastb and g == 0:
                    with scope("wait_gu"):
                        wg_cp.wait()
                        wu_cp.wait()
                        wq_cp.wait()
                    route()
                for MAT in (K, V):
                    if lastb:
                        side = spread(moe1, n1, 0.0, span)
                        if MAT is V:
                            wqtq.pop(0)()
                    elif i == 0:
                        side = spread(lnq, 2 * NLN // 16, lnpos, span) if g >= 4 else []
                    elif i == 1:
                        left = 2 * (G - g) - (MAT is V)
                        side = spread(lnq, -(-len(lnq) // left), lnpos, span) if g >= 2 else []
                    else:
                        side = spread(lnq, -(-NLN // 16), lnpos, span)
                    MAT(i, g, side)
                if len(pend) >= 1:
                    KV(*pend.pop(0))
                pend.append((i, g))
            assert not lnq
        for f in moe1:
            f(None)
        del moe1[:]

        idx, idx16, rmax = rt["idx"], rt["idx16"], rt["rmax"]
        ri = lax.broadcasted_iota(jnp.int32, (128, 128), 0) // DH
        ci = lax.broadcasted_iota(jnp.int32, (128, 128), 1) // DH
        same = ri == ci

        def Mp(g):
            kvb = jnp.where(same, kv[g], 0.0).astype(bf16)
            m32[g * 64:(g + 1) * 64, :] = _pack(_dot(kvb, wo_v[g * 128:(g + 1) * 128, :]))

        def ZC(g):
            z = jnp.sum(zacc[g], axis=0, keepdims=True)
            zc_v[g * 128:(g + 1) * 128, :] = jnp.broadcast_to(z, (128, 128)).T

        def dside(k):
            return spread(moe2, k, 0.0, span)

        def Q(i, t):
            w0 = (i * TM + t * 128) // 2
            xt = _unpack(xn32[w0:w0 + 64, :])
            p = _phi(mm(wqt32[...], xt, dside(2 * n2), nt=True))
            for g in range(G):
                outs = []
                for h in range(4):
                    r0 = g * 128 + h * DH
                    ph = p[r0:r0 + DH, :]
                    tz = ph * zc_v[r0:r0 + DH, :]
                    s8 = jnp.sum(tz.reshape(DH // 8, 8, 128), axis=0)
                    den = jnp.sum(s8, axis=0, keepdims=True) + 1e-6
                    rc = pl.reciprocal(den, approx=True)
                    rc = rc * (2.0 - den * rc)
                    outs.append(ph * rc)
                ot = jnp.concatenate(outs, axis=0).astype(bf16)
                op32[w0:w0 + 64, g * 128:(g + 1) * 128] = pltpu.bitcast(ot.T, u32) | st["zero"][:64]

        def OUT(i, g):
            cols = slice(g * 128, (g + 1) * 128)
            acc = mm(op32[pl.ds(i * TM // 2, TM // 2), :], _unpack(m32[:, cols]), dside(n2))
            res = (x_v[pl.ds(i * TM, TM), cols].astype(f32)
                   + _unpack(xn32[pl.ds(i * TM // 2, TM // 2), cols]).astype(f32))
            out_v[pl.ds(i * TM, TM), cols] = (acc + res).astype(bf16)

        with scope("wait_qod"):
            wo_cp.wait()
            wd_cp.wait()
        for g in range(G - 1):
            ZC(g)
        ZC(G - 1)
        Q(0, 0)
        KV(*pend.pop(0))
        assert not pend
        Mp(0); Mp(1)
        Q(0, 1)
        Mp(2); Mp(3); Mp(4)
        Q(0, 2)
        Mp(5); Mp(6); Mp(7)
        Q(0, 3)

        gate = jax.nn.sigmoid(jnp.full((1, 1), rmax, f32))
        rr = lax.broadcasted_iota(jnp.int32, (16, D), 0)

        def patch(i, cols=slice(None)):
            slab = pl.multiple_of(jnp.clip(idx16, i * TM, (i + 1) * TM - 16), 16)
            cur = out_v[pl.ds(slab, 16), cols]
            upd = (cur.astype(f32) + ys["yg"][:, cols]).astype(bf16)
            out_v[pl.ds(slab, 16), cols] = jnp.where(rr[:, cols] + slab == idx, upd, cur)

        for i in range(NB):
            if i + 1 < NB:
                for t in range(4):
                    Q(i + 1, t)
                    OUT(i, 2 * t)
                    OUT(i, 2 * t + 1)
                if i == 0:
                    for f in moe2:
                        f(None)
                    del moe2[:]
                    ys["yg"] = jnp.broadcast_to(jnp.sum(ys["yv"], axis=0, keepdims=True), (16, D)) * gate
                patch(i)
                o_cp(i).start()
            else:
                for n in range(NW):
                    OUT(i, 2 * n)
                    OUT(i, 2 * n + 1)
                    patch(i, slice(n * W, (n + 1) * W))
                    ol_cp(n).start()
        with scope("wait_out"):
            for i in range(NB - 1):
                o_cp(i).wait()
            for n in range(NW):
                ol_cp(n).wait()

    any_spec = pl.BlockSpec(memory_space=pl.ANY)
    scratch = [
        pltpu.VMEM((S, D), bf16),
        pltpu.VMEM((S // 2, D), u32),
        pltpu.VMEM((D, D), bf16),
        pltpu.VMEM((D, D), bf16),
        pltpu.VMEM((D, D), bf16),
        pltpu.VMEM((D, D), bf16),
        pltpu.VMEM((D // 2, D), u32),
        pltpu.VMEM((S // 2, D), u32),
        pltpu.VMEM((D,), bf16),
        pltpu.VMEM((D, F), bf16),
        pltpu.VMEM((D, F), bf16),
        pltpu.VMEM((F, D), bf16),
        pltpu.VMEM((S, D), bf16),
        pltpu.VMEM((D, 128), f32),
        pltpu.VMEM((F, 128), f32),
        pltpu.VMEM((D // 2, D), u32),
        pltpu.VMEM((D, 128), f32),
        pltpu.SemaphoreType.DMA((X0,)),
        pltpu.SemaphoreType.DMA((S // TM,)),
        pltpu.SemaphoreType.DMA((len(WSL),)),
        pltpu.SemaphoreType.DMA((len(WSL),)),
        pltpu.SemaphoreType.DMA((6,)),
        pltpu.SemaphoreType.DMA((S // TM - 1 + 4,)),
    ]

    def run(A_x, A_wqkv, A_wo, B_x, B_w_r, B_w_gate, B_w_up, B_w_down):
        out = pl.pallas_call(
            kernel,
            out_shape=jax.ShapeDtypeStruct((S, D), bf16),
            in_specs=[any_spec] * 7,
            out_specs=any_spec,
            scratch_shapes=scratch,
            compiler_params=pltpu.CompilerParams(vmem_limit_bytes=120 * 2**20, flags=flags, fuse_transposed_lhs_in_matmul=fuse),
        )(A_x.reshape(S, D), A_wqkv, A_wo, B_w_r, B_w_gate, B_w_up, B_w_down)
        return out.reshape(1, S, D)
    return jax.jit(run)


_run = make_kernel(SL=32,CR=32,X0=2)


@jax.jit
def pallas_parallel_sum__linear_attn_block__moe_arch_mod__prompt_kernel(
    A_x: jax.Array,
    A_wqkv: jax.Array,
    A_wo: jax.Array,
    B_x: jax.Array,
    B_w_r: jax.Array,
    B_w_gate: jax.Array,
    B_w_up: jax.Array,
    B_w_down: jax.Array,
):
    return _run(A_x, A_wqkv, A_wo, B_x, B_w_r, B_w_gate, B_w_up, B_w_down)
```

```python
import functools
import numpy as np
import jax
import jax.numpy as jnp
from jax import lax
from jax.experimental import pallas as pl
from jax.experimental.pallas import tpu as pltpu

S, D, H, DH, F = 2048, 1024, 32, 32, 3584
G = D // 128
f32, bf16, u32 = jnp.float32, jnp.bfloat16, jnp.uint32
EPS_B = 1.00135803e-05
FLAGS = {"XLA_TPU_EVENLY_DISTRIBUTE_CRITICAL_NODES": True}


def _rb(x):
    return x.astype(bf16).astype(f32)


def _phi(t):
    return jnp.where(t > 0, t + 1.0, jnp.exp(t)) + 1e-6


def _dot(a, b):
    return jnp.dot(a, b, preferred_element_type=f32)


def _pack(x):
    return pltpu.bitcast(x.astype(bf16), u32)


def _unpack(w):
    return pltpu.bitcast(w, bf16)


def _bits(x):
    return pltpu.bitcast(x, u32)


def _tiles(x):
    return [x[r:r + 8, c:c + 128] for r in range(0, x.shape[0], 8) for c in range(0, x.shape[1], 128)]


def _or_all(ts):
    return functools.reduce(jnp.bitwise_or, ts)


class _Null:
    def __enter__(self):
        return self
    def __exit__(self, *a):
        return False


def make_kernel(TM=512, CR=32, CH=512, X0=2, KB=16, SL=64, flags=None, scopes=False, moe="vpu",
                lnpos=0.0, lag=0.0, span=0.95, split=True, anchor=True, fuse=False,
                WSL=((0, 1), (1, 1), (2, 2), (4, 2), (6, 2)), NSLOT2=22, kvx=(0, 1, 2), nodma=False, endanch=True, ENDROW=1, ENDK=4, lolate=True, sepw0=True):
    NB = S // TM
    NC = F // CH
    NLN = TM // CR
    XR = TM // X0
    W = 256

    def scope(name):
        return jax.named_scope(name) if scopes else _Null()

    def kernel(x_hbm, wqkv_hbm, wo_hbm, wr_hbm, wg_hbm, wu_hbm, wd_hbm, out_hbm,
               x_v, xn32, wq_v, wk_v, wv_v, wo_v, m32, op32, wr_v, wg_v, wu_v, wd_v, out_v, xb_v, hb_v,
               wqt32, zc_v,
               x0_sem, x_sem, k_sem, v_sem, w_sem, o_sem):
        NW = D // W
        def cp(src, dst, sem):
            return pltpu.make_async_copy(src, dst, sem)
        def x0_cp(c):
            return cp(x_hbm.at[pl.ds(c * XR, XR), :], x_v.at[pl.ds(c * XR, XR), :], x0_sem.at[c])
        def x_cp(i):
            return cp(x_hbm.at[pl.ds(i * TM, TM), :], x_v.at[pl.ds(i * TM, TM), :], x_sem.at[i])
        def x1_cp(h):
            r0 = TM + h * (TM // 2)
            return cp(x_hbm.at[pl.ds(r0, TM // 2), :], x_v.at[pl.ds(r0, TM // 2), :], x_sem.at[h])
        def wk_cp(j):
            g0, ng = WSL[j]
            return cp(wqkv_hbm.at[:, pl.ds(D + g0 * 128, ng * 128)], wk_v.at[:, pl.ds(g0 * 128, ng * 128)], k_sem.at[j])
        def wv_cp(j):
            g0, ng = WSL[j]
            return cp(wqkv_hbm.at[:, pl.ds(2 * D + g0 * 128, ng * 128)], wv_v.at[:, pl.ds(g0 * 128, ng * 128)], v_sem.at[j])
        wq_cp = cp(wqkv_hbm.at[:, pl.ds(0, D)], wq_v, w_sem.at[0])
        wo_cp = cp(wo_hbm, wo_v, w_sem.at[1])
        wr_cp = cp(wr_hbm, wr_v, w_sem.at[2])
        wg_cp = cp(wg_hbm, wg_v, w_sem.at[3])
        wu_cp = cp(wu_hbm, wu_v, w_sem.at[4])
        wd_cp = cp(wd_hbm, wd_v, w_sem.at[5])
        def o_cp(i):
            return cp(out_v.at[pl.ds(i * TM, TM), :], out_hbm.at[pl.ds(i * TM, TM), :], o_sem.at[i])
        def ol_cp(n):
            r0 = (NB - 1) * TM
            return cp(out_v.at[pl.ds(r0, TM), pl.ds(n * W, W)],
                      out_hbm.at[pl.ds(r0, TM), pl.ds(n * W, W)], o_sem.at[NB - 1 + n])

        x0s = [x0_cp(c) for c in range(X0)]
        wks = [wk_cp(j) for j in range(len(WSL))]
        wvs = [wv_cp(j) for j in range(len(WSL))]
        xs_ = {i: x_cp(i) for i in range(2, NB)}
        x1s = [x1_cp(0), x1_cp(1)]
        if X0 == 4:
            queue = {
                "begin": [wr_cp, x0s[0], x0s[1]],
                ("x0", 0): [x0s[2], x0s[3]],
                ("x0", 1): [wks[0], wvs[0]],
                ("x0", 2): [wks[1], wvs[1]],
                ("x0", 3): [wks[2], wvs[2]],
            }
        else:
            queue = {
                "begin": [wr_cp, x0s[0], x0s[1], wks[0], wvs[0]],
                ("x0", 0): [wks[1], wvs[1]],
                ("x0", 1): [wks[2], wvs[2]],
            }
        queue.update({
            ("w", 0): [x1s[0]],
            ("w", 1): [wks[3], wvs[3]],
            ("w", 2): [wks[4], wvs[4], x1s[1]],
            ("w", 3): [xs_[2]],
            ("w", 4): [xs_[3]],
        })
        queue[("w", 0, "lo")] = []
        if nodma:
            tiny = lambda j: cp(wg_hbm.at[pl.ds(0, 16), pl.ds(0, 128)], wg_v.at[pl.ds(16 * j, 16), pl.ds(0, 128)], w_sem.at[j])
            wg_cp, wu_cp, wd_cp = tiny(3), tiny(4), tiny(5)
        if lolate:
            queue[("w", 0, "lo")] = [wq_cp]
            queue[("w", 1, "lo")] = [wg_cp]
            queue[("w", 2, "lo")] = [wu_cp]
            queue[("w", 3, "lo")] = [wo_cp]
            queue[("w", 4, "lo")] = [wd_cp]
        else:
            queue["begin_lo"] = [wq_cp]
            queue[("x0", 0, "lo")] = [wg_cp]
            queue[("w", 0, "lo")] = [wu_cp]
            queue[("w", 1, "lo")] = [wo_cp]
            queue[("w", 2, "lo")] = [wd_cp]
        def kick(key):
            for c_ in queue.pop(key, ()):
                c_.start()
            lo = "begin_lo" if key == "begin" else key + ("lo",)
            for c_ in queue.pop(lo, ()):
                c_.start(priority=1)
        kick("begin")

        st = dict(best=None, bidx=None, endq=[])

        def never(tok):
            return pltpu.bitcast(tok, f32) > st["big"]

        def mm(lhs_w, rhs, side=(), nt=False):
            dn = (((1,), (1,)), ((), ())) if nt else (((1,), (0,)), ((), ()))
            R = lhs_w.shape[0] // 4
            hd = D // 2
            if st["endq"] and not nt:
                tok = _or_all(st["endq"])
                del st["endq"][:]
                rg, kk = lhs_w.shape[0] // 8 - ENDROW, ENDK
                m = pltpu.bitcast(tok, f32) > st["big"]
                blk = lhs_w[rg * 8:(rg + 1) * 8, :]
                tl = blk[:, kk * 128:(kk + 1) * 128]
                tl = jnp.where(m, jnp.zeros_like(tl), tl)
                blk = jnp.concatenate([blk[:, :kk * 128], tl, blk[:, (kk + 1) * 128:]], axis=1) if kk < G - 1 else \
                    jnp.concatenate([blk[:, :kk * 128], tl], axis=1)
                parts = [lhs_w[:rg * 8], blk] + ([lhs_w[(rg + 1) * 8:]] if (rg + 1) * 8 < lhs_w.shape[0] else [])
                lhs_w = jnp.concatenate(parts, axis=0)
            if not side:
                return lax.dot_general(_unpack(lhs_w), rhs, dn, preferred_element_type=f32)
            res = None
            newq = []
            for h in range(2):
                ks = slice(h * hd, (h + 1) * hd)
                part = lax.dot_general(_unpack(lhs_w[:, ks]), rhs[:, ks] if nt else rhs[ks, :], dn,
                                       preferred_element_type=f32)
                for pos, thunk in side:
                    if (pos >= 0.5) == (h == 1):
                        r = min(int((pos * 2 - h) * R), R - 1)
                        t_ = thunk(part[r * 8:(r + 1) * 8, 0:128] if anchor else None)
                        if t_ is not None:
                            newq.append(t_)
                res = part if res is None else res + part
            st["endq"].extend(newq)
            return res

        def gated(x, tok):
            if tok is None:
                return x
            m = tok > st["big"]
            m = jnp.concatenate([m] * (x.shape[1] // 128), axis=1) if x.shape[1] > 128 else m[:, :x.shape[1]]
            m = jnp.concatenate([m] * (x.shape[0] // 8), axis=0) if x.shape[0] > 8 else m
            return jnp.where(m, 0.0, x)

        def spread(q, k, lo=0.0, hi=1.0):
            items = [q.pop(0) for _ in range(min(k, len(q)))]
            return [(lo + (hi - lo) * j / len(items), f) for j, f in enumerate(items)]

        def ln_piece(i, c, tok=None):
            r0 = i * TM + c * CR
            xf = x_v[pl.ds(r0, CR), :].astype(f32)
            mean = gated(jnp.sum(xf, axis=1, keepdims=True), tok) * (1.0 / D)
            mb = _rb(mean)
            d = xf - mb
            dm = mean - mb
            var = jnp.sum(d * d, axis=1, keepdims=True) * (1.0 / D) - dm * dm
            rs = jnp.sum(d * st["wr"], axis=1, keepdims=True)
            inv = 1.0 / _rb(jnp.sqrt(_rb(_rb(var) + EPS_B)))
            r = _rb(rs * inv)
            packed = _pack(d * inv)
            xn32[pl.ds(r0 // 2, CR // 2), :] = packed
            ridx = lax.broadcasted_iota(jnp.int32, (CR, 1), 0) + r0
            if st["best"] is None:
                st["best"], st["bidx"] = r, ridx
            else:
                take = r > st["best"]
                st["best"] = jnp.where(take, r, st["best"])
                st["bidx"] = jnp.where(take, ridx, st["bidx"])
            if endanch and tok is not None:
                return _or_all(_tiles(packed))

        def xw(i):
            return xn32[pl.ds(i * TM // 2, TM // 2), :]

        for c0 in range(X0):
            with scope(f"wait_x0_{c0}"):
                if c0 == 0:
                    wr_cp.wait()
                x0s[c0].wait()
            kick(("x0", c0))
            if c0 == 0:
                st["wr"] = wr_v[...].astype(f32).reshape(1, D)
                wbits = pltpu.bitcast(jnp.broadcast_to(st["wr"][:, 0:128], (8, 128)), jnp.int32)
                one = (wbits | 1) & 1
                st["big"] = pltpu.bitcast(one * 0x7F800000, f32)
                st["zero"] = pltpu.bitcast(jnp.concatenate([(one - 1)] * 8, axis=0), u32)
            for c in range(c0 * NLN // X0, (c0 + 1) * NLN // X0):
                ln_piece(0, c)

        pkb, vb = {}, {}
        kv = [None] * G
        zacc = [None] * G

        def K(i, g, side=()):
            pk = _phi(mm(xw(i), wk_v[:, g * 128:(g + 1) * 128], side))
            zp = jnp.sum(pk.reshape(TM // 8, 8, 128), axis=0)
            zacc[g] = zp if zacc[g] is None else zacc[g] + zp
            pkb[i, g] = pk.astype(bf16)

        def V(i, g, side=()):
            vb[i, g] = mm(xw(i), wv_v[:, g * 128:(g + 1) * 128], side).astype(bf16)

        def KV(i, g):
            if i in kvx:
                kt = pltpu.bitcast(pkb.pop((i, g)).T, u32) | jnp.concatenate([st["zero"][:64]] * (TM // 128), axis=1)
                p = _dot(_unpack(kt), vb.pop((i, g)))
            else:
                p = lax.dot_general(pkb.pop((i, g)), vb.pop((i, g)), (((0,), (0,)), ((), ())),
                                    preferred_element_type=f32)
            kv[g] = p if kv[g] is None else kv[g] + p

        ys = dict(yv=None)

        def col_bcast(dst, k0, row):
            for t in range(row.shape[1] // 128):
                blk = jnp.broadcast_to(row[:, t * 128:(t + 1) * 128], (128, 128))
                dst[pl.ds(k0 + t * 128, 128), :] = blk.T

        def mv_step(accs, b_ref, k0, nk, w_refs, c0, nc, tok=None):
            for kb in range(nk // KB):
                rows = pl.ds(k0 + kb * KB, KB)
                bb = gated(b_ref[rows, :], tok)
                bt = jnp.concatenate([bb] * (nc // 128), axis=1)
                for j, w_ref in enumerate(w_refs):
                    p = w_ref[rows, pl.ds(c0, nc)].astype(f32) * bt
                    p = jnp.sum(p.reshape(KB // 8, 8, nc), axis=0)
                    accs[j] = p if accs[j] is None else accs[j] + p

        def gu_slices(c):
            accs = [None, None]
            out = [functools.partial(mv_step, accs, xb_v, k0, SL, [wg_v, wu_v], c * CH, CH)
                   for k0 in range(0, D, SL)]
            def fin(tok=None):
                gt = jnp.sum(accs[0], axis=0, keepdims=True)
                ut = jnp.sum(accs[1], axis=0, keepdims=True)
                h = _rb(gt * jax.nn.sigmoid(gt) * ut)
                col_bcast(hb_v, c * CH, h)
            return out + [fin]

        def dn_slices(c):
            def step(k0, tok=None):
                accs = [ys["yv"]]
                mv_step(accs, hb_v, k0, SL // 2, [wd_v], 0, D, tok)
                ys["yv"] = accs[0]
            return [functools.partial(step, k0) for k0 in range(c * CH, (c + 1) * CH, SL // 2)]

        def wqt_slab(nt_, tok=None):
            slab = wq_v[:, nt_ * 128:(nt_ + 1) * 128]
            wt = pltpu.bitcast(slab.T, u32)
            wqt32[nt_ * 64:(nt_ + 1) * 64, :] = wt | jnp.concatenate([st["zero"]] * G, axis=1)
        wqtq = [functools.partial(wqt_slab, j) for j in range(G)]

        moe1 = [f for c in range(NC) for f in gu_slices(c)]
        moe2 = [f for c in range(NC) for f in dn_slices(c)]
        n1 = -(-len(moe1) // 16)
        n2 = -(-len(moe2) // NSLOT2)

        rt = {}
        def route():
            best, bidx = st["best"], st["bidx"]
            rmax = jnp.max(best)
            idx = jnp.min(jnp.where(best == rmax, bidx, S))
            idx = jnp.minimum(idx, S - 1)
            idx16 = pl.multiple_of((idx // 16) * 16, 16)
            rt.update(rmax=rmax, idx=idx, idx16=idx16)
            slab = _unpack(xn32[pl.ds(pl.multiple_of(idx16 // 2, 8), 8), :])
            rr16 = lax.broadcasted_iota(jnp.int32, (16, D), 0)
            xrow = jnp.sum(jnp.where(rr16 == idx - idx16, slab.astype(f32), 0.0), axis=0, keepdims=True)
            col_bcast(xb_v, 0, xrow)

        pend = []
        for i in range(NB):
            lastb = i == NB - 1
            lnq = [] if lastb else [functools.partial(ln_piece, i + 1, c) for c in range(NLN)]
            for g in range(G):
                n = g // 2
                if i == 0:
                    for j, (g0, ng) in enumerate(WSL):
                        if g == g0:
                            with scope(f"wait_w{j}"):
                                wks[j].wait()
                                if not (sepw0 and j == 0):
                                    wvs[j].wait()
                                if g == 4:
                                    x1s[0].wait()
                                if g == 6:
                                    x1s[1].wait()
                            kick(("w", j))
                if i == 1 and g == 2:
                    with scope("wait_x"):
                        for j in range(2, NB):
                            xs_[j].wait()
                if lastb and g == 0:
                    with scope("wait_gu"):
                        wg_cp.wait()
                        wu_cp.wait()
                        wq_cp.wait()
                    route()
                for MAT in (K, V):
                    if sepw0 and i == 0 and g == 0 and MAT is V:
                        with scope("wait_wv0"):
                            wvs[0].wait()
                    if lastb:
                        side = spread(moe1, n1, 0.0, span)
                        if MAT is V:
                            wqtq.pop(0)()
                    elif i == 0:
                        side = spread(lnq, 2 * NLN // 16, lnpos, span) if g >= 4 else []
                    elif i == 1:
                        left = 2 * (G - g) - (MAT is V)
                        side = spread(lnq, -(-len(lnq) // left), lnpos, span) if g >= 2 else []
                    else:
                        side = spread(lnq, -(-NLN // 16), lnpos, span)
                    MAT(i, g, side)
                if len(pend) >= 1:
                    KV(*pend.pop(0))
                pend.append((i, g))
            assert not lnq
        for f in moe1:
            f(None)
        del moe1[:]

        idx, idx16, rmax = rt["idx"], rt["idx16"], rt["rmax"]
        ri = lax.broadcasted_iota(jnp.int32, (128, 128), 0) // DH
        ci = lax.broadcasted_iota(jnp.int32, (128, 128), 1) // DH
        same = ri == ci

        def Mp(g):
            kvb = jnp.where(same, kv[g], 0.0).astype(bf16)
            m32[g * 64:(g + 1) * 64, :] = _pack(_dot(kvb, wo_v[g * 128:(g + 1) * 128, :]))

        def ZC(g):
            z = jnp.sum(zacc[g], axis=0, keepdims=True)
            zc_v[g * 128:(g + 1) * 128, :] = jnp.broadcast_to(z, (128, 128)).T

        def dside(k):
            return spread(moe2, k, 0.0, span)

        def Q(i, t):
            w0 = (i * TM + t * 128) // 2
            xt = _unpack(xn32[w0:w0 + 64, :])
            p = _phi(mm(wqt32[...], xt, dside(2 * n2), nt=True))
            for g in range(G):
                outs = []
                for h in range(4):
                    r0 = g * 128 + h * DH
                    ph = p[r0:r0 + DH, :]
                    tz = ph * zc_v[r0:r0 + DH, :]
                    s8 = jnp.sum(tz.reshape(DH // 8, 8, 128), axis=0)
                    den = jnp.sum(s8, axis=0, keepdims=True) + 1e-6
                    rc = pl.reciprocal(den, approx=True)
                    rc = rc * (2.0 - den * rc)
                    outs.append(ph * rc)
                ot = jnp.concatenate(outs, axis=0).astype(bf16)
                op32[w0:w0 + 64, g * 128:(g + 1) * 128] = pltpu.bitcast(ot.T, u32) | st["zero"][:64]

        def OUT(i, g):
            cols = slice(g * 128, (g + 1) * 128)
            acc = mm(op32[pl.ds(i * TM // 2, TM // 2), :], _unpack(m32[:, cols]), dside(n2))
            res = (x_v[pl.ds(i * TM, TM), cols].astype(f32)
                   + _unpack(xn32[pl.ds(i * TM // 2, TM // 2), cols]).astype(f32))
            out_v[pl.ds(i * TM, TM), cols] = (acc + res).astype(bf16)

        with scope("wait_qod"):
            wo_cp.wait()
            wd_cp.wait()
        for g in range(G - 1):
            ZC(g)
        ZC(G - 1)
        Q(0, 0)
        KV(*pend.pop(0))
        assert not pend
        Mp(0); Mp(1)
        Q(0, 1)
        Mp(2); Mp(3); Mp(4)
        Q(0, 2)
        Mp(5); Mp(6); Mp(7)
        Q(0, 3)

        gate = jax.nn.sigmoid(jnp.full((1, 1), rmax, f32))
        rr = lax.broadcasted_iota(jnp.int32, (16, D), 0)

        def patch(i, cols=slice(None)):
            slab = pl.multiple_of(jnp.clip(idx16, i * TM, (i + 1) * TM - 16), 16)
            cur = out_v[pl.ds(slab, 16), cols]
            upd = (cur.astype(f32) + ys["yg"][:, cols]).astype(bf16)
            out_v[pl.ds(slab, 16), cols] = jnp.where(rr[:, cols] + slab == idx, upd, cur)

        for i in range(NB):
            if i + 1 < NB:
                for t in range(4):
                    Q(i + 1, t)
                    OUT(i, 2 * t)
                    OUT(i, 2 * t + 1)
                if i == 0:
                    for f in moe2:
                        f(None)
                    del moe2[:]
                    ys["yg"] = jnp.broadcast_to(jnp.sum(ys["yv"], axis=0, keepdims=True), (16, D)) * gate
                patch(i)
                o_cp(i).start()
            else:
                for n in range(NW):
                    OUT(i, 2 * n)
                    OUT(i, 2 * n + 1)
                    patch(i, slice(n * W, (n + 1) * W))
                    ol_cp(n).start()
        with scope("wait_out"):
            for i in range(NB - 1):
                o_cp(i).wait()
            for n in range(NW):
                ol_cp(n).wait()

    any_spec = pl.BlockSpec(memory_space=pl.ANY)
    scratch = [
        pltpu.VMEM((S, D), bf16),
        pltpu.VMEM((S // 2, D), u32),
        pltpu.VMEM((D, D), bf16),
        pltpu.VMEM((D, D), bf16),
        pltpu.VMEM((D, D), bf16),
        pltpu.VMEM((D, D), bf16),
        pltpu.VMEM((D // 2, D), u32),
        pltpu.VMEM((S // 2, D), u32),
        pltpu.VMEM((D,), bf16),
        pltpu.VMEM((D, F), bf16),
        pltpu.VMEM((D, F), bf16),
        pltpu.VMEM((F, D), bf16),
        pltpu.VMEM((S, D), bf16),
        pltpu.VMEM((D, 128), f32),
        pltpu.VMEM((F, 128), f32),
        pltpu.VMEM((D // 2, D), u32),
        pltpu.VMEM((D, 128), f32),
        pltpu.SemaphoreType.DMA((X0,)),
        pltpu.SemaphoreType.DMA((S // TM,)),
        pltpu.SemaphoreType.DMA((len(WSL),)),
        pltpu.SemaphoreType.DMA((len(WSL),)),
        pltpu.SemaphoreType.DMA((6,)),
        pltpu.SemaphoreType.DMA((S // TM - 1 + 4,)),
    ]

    def run(A_x, A_wqkv, A_wo, B_x, B_w_r, B_w_gate, B_w_up, B_w_down):
        out = pl.pallas_call(
            kernel,
            out_shape=jax.ShapeDtypeStruct((S, D), bf16),
            in_specs=[any_spec] * 7,
            out_specs=any_spec,
            scratch_shapes=scratch,
            compiler_params=pltpu.CompilerParams(vmem_limit_bytes=120 * 2**20, flags=flags, fuse_transposed_lhs_in_matmul=fuse),
        )(A_x.reshape(S, D), A_wqkv, A_wo, B_w_r, B_w_gate, B_w_up, B_w_down)
        return out.reshape(1, S, D)
    return jax.jit(run)


_run = make_kernel(SL=32,CR=32,X0=4)


@jax.jit
def pallas_parallel_sum__linear_attn_block__moe_arch_mod__prompt_kernel(
    A_x: jax.Array,
    A_wqkv: jax.Array,
    A_wo: jax.Array,
    B_x: jax.Array,
    B_w_r: jax.Array,
    B_w_gate: jax.Array,
    B_w_up: jax.Array,
    B_w_down: jax.Array,
):
    return _run(A_x, A_wqkv, A_wo, B_x, B_w_r, B_w_gate, B_w_up, B_w_down)
```

```python
import functools

import jax
import jax.numpy as jnp
from jax import lax
from jax.experimental import pallas as pl
from jax.experimental.pallas import tpu as pltpu

S, D, H, DH, F = 2048, 1024, 32, 32, 3584
G = D // 128
TM = 512
NB = S // TM
CR = 32
NLN = TM // CR
X0 = 4
XR = TM // X0
CH = 512
NC = F // CH
KB = 16
SL = 32
NSLOT2 = 20
WSL = ((0, 1), (1, 1), (2, 2), (4, 2), (6, 2))
EPS_B = 1.00135803e-05

f32, bf16, u32, i32 = jnp.float32, jnp.bfloat16, jnp.uint32, jnp.int32
NN = (((1,), (0,)), ((), ()))
NT = (((1,), (1,)), ((), ()))
TN = (((0,), (0,)), ((), ()))


def _rb(x):
    return x.astype(bf16).astype(f32)


def _phi(t):
    return jnp.where(t > 0, t + 1.0, jnp.exp(t)) + 1e-6


def _dot(a, b, dims=NN):
    return lax.dot_general(a, b, dims, preferred_element_type=f32)


def _pack(x):
    return pltpu.bitcast(x.astype(bf16), u32)


def _unpack(w):
    return pltpu.bitcast(w, bf16)


def _or_tiles(x):
    tiles = [x[r:r + 8, c:c + 128] for r in range(0, x.shape[0], 8) for c in range(0, x.shape[1], 128)]
    return functools.reduce(jnp.bitwise_or, tiles)


def _kernel(x_hbm, wqkv_hbm, wo_hbm, wr_hbm, wg_hbm, wu_hbm, wd_hbm, out_hbm,
            x_v, xn32, wq_v, wk_v, wv_v, wo_v, m32, op32, wr_v, wg_v, wu_v, wd_v, out_v,
            xb_v, hb_v, wqt32, zc_v,
            x0_sem, x_sem, k_sem, v_sem, w_sem, o_sem):
    cp = pltpu.make_async_copy

    def rows_cp(hbm, vmem, r0, n, sem):
        return cp(hbm.at[pl.ds(r0, n), :], vmem.at[pl.ds(r0, n), :], sem)

    def slab_cp(base, dst, j, sem):
        g0, ng = WSL[j]
        return cp(wqkv_hbm.at[:, pl.ds(base + g0 * 128, ng * 128)], dst.at[:, pl.ds(g0 * 128, ng * 128)], sem.at[j])

    x0s = [rows_cp(x_hbm, x_v, c * XR, XR, x0_sem.at[c]) for c in range(X0)]
    x1s = [rows_cp(x_hbm, x_v, TM + h * (TM // 2), TM // 2, x_sem.at[h]) for h in range(2)]
    xs = {i: rows_cp(x_hbm, x_v, i * TM, TM, x_sem.at[i]) for i in range(2, NB)}
    wks = [slab_cp(D, wk_v, j, k_sem) for j in range(len(WSL))]
    wvs = [slab_cp(2 * D, wv_v, j, v_sem) for j in range(len(WSL))]
    wq_cp = cp(wqkv_hbm.at[:, pl.ds(0, D)], wq_v, w_sem.at[0])
    wo_cp = cp(wo_hbm, wo_v, w_sem.at[1])
    wr_cp = cp(wr_hbm, wr_v, w_sem.at[2])
    wg_cp = cp(wg_hbm, wg_v, w_sem.at[3])
    wu_cp = cp(wu_hbm, wu_v, w_sem.at[4])
    wd_cp = cp(wd_hbm, wd_v, w_sem.at[5])
    outs = [cp(out_v.at[pl.ds(i * TM, TM), :], out_hbm.at[pl.ds(i * TM, TM), :], o_sem.at[i])
            for i in range(NB - 1)]
    last0 = (NB - 1) * TM
    outs_last = [cp(out_v.at[pl.ds(last0, TM), pl.ds(g * 128, 128)],
                    out_hbm.at[pl.ds(last0, TM), pl.ds(g * 128, 128)], o_sem.at[NB - 1 + g])
                 for g in range(G)]

    queue = {
        "begin": [wr_cp, x0s[0], x0s[1]],
        ("x0", 0): [x0s[2], x0s[3]],
        ("x0", 1): [wks[0], wvs[0]],
        ("x0", 2): [wks[1], wvs[1]],
        ("x0", 3): [wks[2], wvs[2]],
        ("w", 0): [x1s[0]],
        ("w", 1): [wks[3], wvs[3]],
        ("w", 2): [wks[4], wvs[4], x1s[1]],
        ("w", 3): [xs[2]],
        ("w", 4): [xs[3]],
    }
    late = {("w", 0): wq_cp, ("w", 1): wg_cp, ("w", 2): wu_cp, ("w", 3): wo_cp, ("w", 4): wd_cp}

    def kick(key):
        for c in queue.pop(key, ()):
            c.start()
        if key in late:
            late.pop(key).start(priority=1)

    kick("begin")

    st = dict(best=None, bidx=None, prev=None, done=[], pending=[])

    def never(tok):
        return (tok if tok.dtype == f32 else pltpu.bitcast(tok, f32)) > st["big"]

    def gated(x, tok):
        if tok is None:
            return x
        m = never(tok)
        m = jnp.concatenate([m] * (x.shape[1] // 128), axis=1) if x.shape[1] > 128 else m[:, :x.shape[1]]
        m = jnp.concatenate([m] * (x.shape[0] // 8), axis=0) if x.shape[0] > 8 else m
        return jnp.where(m, 0.0, x)

    def mm(lhs_w, rhs, side=(), dims=NN):
        tiles = lhs_w.shape[0] // 4
        st["done"] += st["pending"]
        st["pending"] = []
        if st["done"] and dims is NN:
            rg, kk = lhs_w.shape[0] // 16, G // 2
            m = never(functools.reduce(jnp.bitwise_or, st["done"]))
            st["done"] = []
            blk = lhs_w[rg * 8:(rg + 1) * 8, :]
            tl = jnp.where(m, jnp.zeros((8, 128), u32), blk[:, kk * 128:(kk + 1) * 128])
            blk = jnp.concatenate([blk[:, :kk * 128], tl, blk[:, (kk + 1) * 128:]], axis=1)
            lhs_w = jnp.concatenate([lhs_w[:rg * 8], blk, lhs_w[(rg + 1) * 8:]], axis=0)

        def run(todo, src, scale, off):
            for pos, f in todo:
                r = min(int((pos - off) * scale * tiles), tiles - 1)
                t = f(src[r * 8:(r + 1) * 8, 0:128])
                if t is not None:
                    st["pending"].append(t)

        if not side:
            res = _dot(_unpack(lhs_w), rhs, dims)
        elif len(side) <= 2 and dims is NN and st["prev"] is not None:
            run(side, st["prev"], 1.0, 0.0)
            res = _dot(_unpack(lhs_w), rhs, dims)
        else:
            res = None
            for h in range(2):
                ks = slice(h * (D // 2), (h + 1) * (D // 2))
                part = _dot(_unpack(lhs_w[:, ks]), rhs[:, ks] if dims is NT else rhs[ks, :], dims)
                run([(p, f) for p, f in side if (p >= 0.5) == (h == 1)], part, 2.0, 0.5 * h)
                res = part if res is None else res + part
            st["done"] += st["pending"]
            st["pending"] = []
        st["prev"] = res
        return res

    def spread(q, k):
        items = [q.pop(0) for _ in range(min(k, len(q)))]
        return [(0.95 * j / len(items), f) for j, f in enumerate(items)]

    def ln_piece(i, c, tok=None):
        r0 = i * TM + c * CR
        xf = x_v[pl.ds(r0, CR), :].astype(f32)
        mean = gated(jnp.sum(xf, axis=1, keepdims=True), tok) * (1.0 / D)
        mb = _rb(mean)
        d = xf - mb
        dm = mean - mb
        var = jnp.sum(d * d, axis=1, keepdims=True) * (1.0 / D) - dm * dm
        rs = jnp.sum(d * st["wr"], axis=1, keepdims=True)
        inv = 1.0 / _rb(jnp.sqrt(_rb(_rb(var) + EPS_B)))
        r = _rb(rs * inv)
        packed = _pack(d * inv)
        xn32[pl.ds(r0 // 2, CR // 2), :] = packed
        ridx = lax.broadcasted_iota(i32, (CR, 1), 0) + r0
        if st["best"] is None:
            st["best"], st["bidx"] = r, ridx
        else:
            take = r > st["best"]
            st["best"] = jnp.where(take, r, st["best"])
            st["bidx"] = jnp.where(take, ridx, st["bidx"])
        return None if tok is None else _or_tiles(packed)

    def xw(i):
        return xn32[pl.ds(i * TM // 2, TM // 2), :]

    for c0 in range(X0):
        if c0 == 0:
            wr_cp.wait()
        x0s[c0].wait()
        kick(("x0", c0))
        if c0 == 0:
            st["wr"] = wr_v[...].astype(f32).reshape(1, D)
            one = (pltpu.bitcast(jnp.broadcast_to(st["wr"][:, 0:128], (8, 128)), i32) | 1) & 1
            st["big"] = pltpu.bitcast(one * 0x7F800000, f32)
            st["zero"] = pltpu.bitcast(jnp.concatenate([one - 1] * 8, axis=0), u32)
        for c in range(c0 * NLN // X0, (c0 + 1) * NLN // X0):
            ln_piece(0, c)

    pkb, vb = {}, {}
    kv = [None] * G
    zacc = [None] * G

    def K(i, g, side):
        pk = _phi(mm(xw(i), wk_v[:, g * 128:(g + 1) * 128], side))
        zp = jnp.sum(pk.reshape(TM // 8, 8, 128), axis=0)
        zacc[g] = zp if zacc[g] is None else zacc[g] + zp
        pkb[i, g] = pk.astype(bf16)

    def V(i, g, side):
        vb[i, g] = mm(xw(i), wv_v[:, g * 128:(g + 1) * 128], side).astype(bf16)

    def KV(i, g):
        if i < NB - 1:
            zero = jnp.concatenate([st["zero"]] * (TM // 128), axis=1)
            p = _dot(_unpack(pltpu.bitcast(pkb.pop((i, g)).T, u32) | zero), vb.pop((i, g)))
        else:
            p = _dot(pkb.pop((i, g)), vb.pop((i, g)), TN)
        kv[g] = p if kv[g] is None else kv[g] + p

    ys = dict(yv=None)
    rt = {}

    def col_bcast(dst, k0, row):
        for t in range(row.shape[1] // 128):
            dst[pl.ds(k0 + t * 128, 128), :] = jnp.broadcast_to(row[:, t * 128:(t + 1) * 128], (128, 128)).T

    def route():
        best, bidx = st["best"], st["bidx"]
        rmax = jnp.max(best)
        idx = jnp.minimum(jnp.min(jnp.where(best == rmax, bidx, S)), S - 1)
        idx16 = pl.multiple_of((idx // 16) * 16, 16)
        rt.update(rmax=rmax, idx=idx, idx16=idx16)
        slab = _unpack(xn32[pl.ds(pl.multiple_of(idx16 // 2, 8), 8), :]).astype(f32)
        pick = lax.broadcasted_iota(i32, (16, D), 0) == idx - idx16
        col_bcast(xb_v, 0, jnp.sum(jnp.where(pick, slab, 0.0), axis=0, keepdims=True))

    def mv_step(accs, b_ref, k0, nk, w_refs, c0, nc, tok=None):
        for kb in range(nk // KB):
            rows = pl.ds(k0 + kb * KB, KB)
            bt = jnp.concatenate([gated(b_ref[rows, :], tok)] * (nc // 128), axis=1)
            for j, w_ref in enumerate(w_refs):
                p = w_ref[rows, pl.ds(c0, nc)].astype(f32) * bt
                p = jnp.sum(p.reshape(KB // 8, 8, nc), axis=0)
                accs[j] = p if accs[j] is None else accs[j] + p

    def gu_slices(c):
        accs = [None, None]

        def fin(tok=None):
            gt = jnp.sum(accs[0], axis=0, keepdims=True)
            ut = jnp.sum(accs[1], axis=0, keepdims=True)
            col_bcast(hb_v, c * CH, _rb(gt * jax.nn.sigmoid(gt) * ut))

        return [functools.partial(mv_step, accs, xb_v, k0, SL, [wg_v, wu_v], c * CH, CH)
                for k0 in range(0, D, SL)] + [fin]

    def dn_step(k0, tok=None):
        accs = [ys["yv"]]
        mv_step(accs, hb_v, k0, SL // 2, [wd_v], 0, D, tok)
        ys["yv"] = accs[0]

    def wqt_slab(j):
        wt = pltpu.bitcast(wq_v[:, j * 128:(j + 1) * 128].T, u32)
        wqt32[j * 64:(j + 1) * 64, :] = wt | jnp.concatenate([st["zero"]] * G, axis=1)

    moe1 = [f for c in range(NC) for f in gu_slices(c)]
    moe2 = [functools.partial(dn_step, k0) for k0 in range(0, F, SL // 2)]
    n1 = -(-len(moe1) // (2 * G))
    n2 = -(-len(moe2) // NSLOT2)

    pend = []
    for i in range(NB):
        lastb = i == NB - 1
        lnq = [] if lastb else [functools.partial(ln_piece, i + 1, c) for c in range(NLN)]
        for g in range(G):
            if i == 0:
                for j, (g0, _) in enumerate(WSL):
                    if g == g0:
                        wks[j].wait()
                        if j > 0:
                            wvs[j].wait()
                        if g == 4:
                            x1s[0].wait()
                        if g == 6:
                            x1s[1].wait()
                        kick(("w", j))
            if i == 1 and g == 2:
                for j in range(2, NB):
                    xs[j].wait()
            if lastb and g == 0:
                wg_cp.wait()
                wu_cp.wait()
                wq_cp.wait()
                route()
            for m, MAT in enumerate((K, V)):
                if i == 0 and g == 0 and m == 1:
                    wvs[0].wait()
                if lastb:
                    side = spread(moe1, n1)
                    if m == 1:
                        wqt_slab(g)
                elif i == 0:
                    side = spread(lnq, NLN // 8) if g >= 4 else []
                elif i == 1:
                    side = spread(lnq, -(-len(lnq) // (2 * (G - g) - m))) if g >= 2 else []
                else:
                    side = spread(lnq, NLN // (2 * G))
                MAT(i, g, side)
            pend.append((i, g))
        assert not lnq
        if not lastb:
            while pend:
                KV(*pend.pop(0))
    assert not moe1

    idx, idx16, rmax = rt["idx"], rt["idx16"], rt["rmax"]
    same = lax.broadcasted_iota(i32, (128, 128), 0) // DH == lax.broadcasted_iota(i32, (128, 128), 1) // DH

    def Mp(g):
        kvb = jnp.where(same, kv[g], 0.0).astype(bf16)
        m32[g * 64:(g + 1) * 64, :] = _pack(_dot(kvb, wo_v[g * 128:(g + 1) * 128, :]))

    def ZC(g):
        z = jnp.sum(zacc[g], axis=0, keepdims=True)
        zc_v[g * 128:(g + 1) * 128, :] = jnp.broadcast_to(z, (128, 128)).T

    def Q(i, t):
        w0 = (i * TM + t * 128) // 2
        p = _phi(mm(wqt32[...], _unpack(xn32[w0:w0 + 64, :]), spread(moe2, 2 * n2), NT))
        for g in range(G):
            heads = []
            for h in range(4):
                r0 = g * 128 + h * DH
                ph = p[r0:r0 + DH, :]
                tz = ph * zc_v[r0:r0 + DH, :]
                den = jnp.sum(jnp.sum(tz.reshape(DH // 8, 8, 128), axis=0), axis=0, keepdims=True) + 1e-6
                rc = pl.reciprocal(den, approx=True)
                rc = rc * (2.0 - den * rc)
                heads.append(ph * rc)
            ot = jnp.concatenate(heads, axis=0).astype(bf16)
            op32[w0:w0 + 64, g * 128:(g + 1) * 128] = pltpu.bitcast(ot.T, u32) | st["zero"]

    def OUT(i, g):
        cols = slice(g * 128, (g + 1) * 128)
        acc = mm(op32[pl.ds(i * TM // 2, TM // 2), :], _unpack(m32[:, cols]), spread(moe2, n2))
        res = (x_v[pl.ds(i * TM, TM), cols].astype(f32)
               + _unpack(xn32[pl.ds(i * TM // 2, TM // 2), cols]).astype(f32))
        out_v[pl.ds(i * TM, TM), cols] = (acc + res).astype(bf16)

    rr = lax.broadcasted_iota(i32, (16, D), 0)

    def patch(i, cols=slice(None)):
        slab = pl.multiple_of(jnp.clip(idx16, i * TM, (i + 1) * TM - 16), 16)
        cur = out_v[pl.ds(slab, 16), cols]
        upd = (cur.astype(f32) + ys["yg"][:, cols]).astype(bf16)
        out_v[pl.ds(slab, 16), cols] = jnp.where(rr[:, cols] + slab == idx, upd, cur)

    wo_cp.wait()
    wd_cp.wait()
    for g in range(G):
        ZC(g)
    for _ in range(4):
        KV(*pend.pop(0))
    Q(0, 0)
    while pend:
        KV(*pend.pop(0))
    Mp(0); Mp(1)
    Q(0, 1)
    Mp(2); Mp(3); Mp(4)
    Q(0, 2)
    Mp(5); Mp(6); Mp(7)
    Q(0, 3)

    for i in range(NB - 1):
        for t in range(4):
            Q(i + 1, t)
            OUT(i, 2 * t)
            OUT(i, 2 * t + 1)
        if i == 0:
            while moe2:
                moe2.pop(0)()
            gate = jax.nn.sigmoid(jnp.full((1, 1), rmax, f32))
            ys["yg"] = jnp.broadcast_to(jnp.sum(ys["yv"], axis=0, keepdims=True), (16, D)) * gate
        patch(i)
        outs[i].start()
    for g in range(G):
        OUT(NB - 1, g)
        patch(NB - 1, slice(g * 128, (g + 1) * 128))
        outs_last[g].start()
    for c in outs + outs_last:
        c.wait()
    assert not queue and not late


def make_kernel():
    any_spec = pl.BlockSpec(memory_space=pl.ANY)
    scratch = [
        pltpu.VMEM((S, D), bf16),
        pltpu.VMEM((S // 2, D), u32),
        pltpu.VMEM((D, D), bf16),
        pltpu.VMEM((D, D), bf16),
        pltpu.VMEM((D, D), bf16),
        pltpu.VMEM((D, D), bf16),
        pltpu.VMEM((D // 2, D), u32),
        pltpu.VMEM((S // 2, D), u32),
        pltpu.VMEM((D,), bf16),
        pltpu.VMEM((D, F), bf16),
        pltpu.VMEM((D, F), bf16),
        pltpu.VMEM((F, D), bf16),
        pltpu.VMEM((S, D), bf16),
        pltpu.VMEM((D, 128), f32),
        pltpu.VMEM((F, 128), f32),
        pltpu.VMEM((D // 2, D), u32),
        pltpu.VMEM((D, 128), f32),
        pltpu.SemaphoreType.DMA((X0,)),
        pltpu.SemaphoreType.DMA((NB,)),
        pltpu.SemaphoreType.DMA((len(WSL),)),
        pltpu.SemaphoreType.DMA((len(WSL),)),
        pltpu.SemaphoreType.DMA((6,)),
        pltpu.SemaphoreType.DMA((NB - 1 + G,)),
    ]

    def run(A_x, A_wqkv, A_wo, B_x, B_w_r, B_w_gate, B_w_up, B_w_down):
        del B_x
        out = pl.pallas_call(
            _kernel,
            out_shape=jax.ShapeDtypeStruct((S, D), bf16),
            in_specs=[any_spec] * 7,
            out_specs=any_spec,
            scratch_shapes=scratch,
            compiler_params=pltpu.CompilerParams(vmem_limit_bytes=120 * 2**20),
        )(A_x.reshape(S, D), A_wqkv, A_wo, B_w_r, B_w_gate, B_w_up, B_w_down)
        return out.reshape(1, S, D)
    return jax.jit(run)


_run = make_kernel()


@jax.jit
def pallas_parallel_sum__linear_attn_block__moe_arch_mod__prompt_kernel(
    A_x: jax.Array,
    A_wqkv: jax.Array,
    A_wo: jax.Array,
    B_x: jax.Array,
    B_w_r: jax.Array,
    B_w_gate: jax.Array,
    B_w_up: jax.Array,
    B_w_down: jax.Array,
):
    return _run(A_x, A_wqkv, A_wo, B_x, B_w_r, B_w_gate, B_w_up, B_w_down)
```

```python
import functools

import jax
import jax.numpy as jnp
from jax import lax
from jax.experimental import pallas as pl
from jax.experimental.pallas import tpu as pltpu

S, D, H, DH, F = 2048, 1024, 32, 32, 3584
G = D // 128
TM = 512
NB = S // TM
CR = 32
NLN = TM // CR
X0 = 4
XR = TM // X0
CH = 512
NC = F // CH
KB = 16
SL = 32
NSLOT2 = 20
WSL = ((0, 1), (1, 1), (2, 2), (4, 2), (6, 2))
EPS_B = 1.00135803e-05

f32, bf16, u32, i32 = jnp.float32, jnp.bfloat16, jnp.uint32, jnp.int32
NN = (((1,), (0,)), ((), ()))
NT = (((1,), (1,)), ((), ()))
TN = (((0,), (0,)), ((), ()))


def _rb(x):
    return x.astype(bf16).astype(f32)


def _phi(t):
    return jnp.where(t > 0, t + 1.0, jnp.exp(t)) + 1e-6


def _dot(a, b, dims=NN):
    return lax.dot_general(a, b, dims, preferred_element_type=f32)


def _pack(x):
    return pltpu.bitcast(x.astype(bf16), u32)


def _unpack(w):
    return pltpu.bitcast(w, bf16)


def _or_tiles(x):
    tiles = [x[r:r + 8, c:c + 128] for r in range(0, x.shape[0], 8) for c in range(0, x.shape[1], 128)]
    return functools.reduce(jnp.bitwise_or, tiles)


def _kernel(x_hbm, wqkv_hbm, wo_hbm, wr_hbm, wg_hbm, wu_hbm, wd_hbm, out_hbm,
            x_v, xn32, wq_v, wk_v, wv_v, wo_v, m32, op32, wr_v, wg_v, wu_v, wd_v, out_v,
            xb_v, hb_v, wqt32, zc_v,
            x0_sem, x_sem, k_sem, v_sem, w_sem, o_sem):
    cp = pltpu.make_async_copy

    def rows_cp(hbm, vmem, r0, n, sem):
        return cp(hbm.at[pl.ds(r0, n), :], vmem.at[pl.ds(r0, n), :], sem)

    def slab_cp(base, dst, j, sem):
        g0, ng = WSL[j]
        return cp(wqkv_hbm.at[:, pl.ds(base + g0 * 128, ng * 128)], dst.at[:, pl.ds(g0 * 128, ng * 128)], sem.at[j])

    x0s = [rows_cp(x_hbm, x_v, c * XR, XR, x0_sem.at[c]) for c in range(X0)]
    x1s = [rows_cp(x_hbm, x_v, TM + h * (TM // 2), TM // 2, x_sem.at[h]) for h in range(2)]
    xs = {i: rows_cp(x_hbm, x_v, i * TM, TM, x_sem.at[i]) for i in range(2, NB)}
    wks = [slab_cp(D, wk_v, j, k_sem) for j in range(len(WSL))]
    wvs = [slab_cp(2 * D, wv_v, j, v_sem) for j in range(len(WSL))]
    wq_cp = cp(wqkv_hbm.at[:, pl.ds(0, D)], wq_v, w_sem.at[0])
    wo_cp = cp(wo_hbm, wo_v, w_sem.at[1])
    wr_cp = cp(wr_hbm, wr_v, w_sem.at[2])
    wg_cp = cp(wg_hbm, wg_v, w_sem.at[3])
    wu_cp = cp(wu_hbm, wu_v, w_sem.at[4])
    wd_cp = cp(wd_hbm, wd_v, w_sem.at[5])
    outs = [cp(out_v.at[pl.ds(i * TM, TM), :], out_hbm.at[pl.ds(i * TM, TM), :], o_sem.at[i])
            for i in range(NB - 1)]
    last0 = (NB - 1) * TM
    outs_last = [cp(out_v.at[pl.ds(last0, TM), pl.ds(g * 128, 128)],
                    out_hbm.at[pl.ds(last0, TM), pl.ds(g * 128, 128)], o_sem.at[NB - 1 + g])
                 for g in range(G)]

    queue = {
        "begin": [wr_cp, x0s[0], x0s[1]],
        ("x0", 0): [x0s[2], x0s[3]],
        ("x0", 1): [wks[0], wvs[0]],
        ("x0", 2): [wks[1], wvs[1]],
        ("x0", 3): [wks[2], wvs[2]],
        ("w", 0): [x1s[0]],
        ("w", 1): [wks[3], wvs[3]],
        ("w", 2): [wks[4], wvs[4], x1s[1]],
        ("w", 3): [xs[2]],
        ("w", 4): [xs[3]],
    }
    late = {("w", 0): wq_cp, ("w", 1): wg_cp, ("w", 2): wu_cp, ("w", 3): wo_cp, ("w", 4): wd_cp}

    def kick(key):
        for c in queue.pop(key, ()):
            c.start()
        if key in late:
            late.pop(key).start(priority=1)

    kick("begin")

    st = dict(best=None, bidx=None, prev=None, done=[], pending=[])

    def never(tok):
        return (tok if tok.dtype == f32 else pltpu.bitcast(tok, f32)) > st["big"]

    def gated(x, tok):
        if tok is None:
            return x
        m = never(tok)
        m = jnp.concatenate([m] * (x.shape[1] // 128), axis=1) if x.shape[1] > 128 else m[:, :x.shape[1]]
        m = jnp.concatenate([m] * (x.shape[0] // 8), axis=0) if x.shape[0] > 8 else m
        return jnp.where(m, 0.0, x)

    def mm(lhs_w, rhs, side=(), dims=NN):
        tiles = lhs_w.shape[0] // 4
        st["done"] += st["pending"]
        st["pending"] = []
        if st["done"] and dims is NN:
            rg, kk = lhs_w.shape[0] // 16, G // 2
            m = never(functools.reduce(jnp.bitwise_or, st["done"]))
            st["done"] = []
            blk = lhs_w[rg * 8:(rg + 1) * 8, :]
            tl = jnp.where(m, jnp.zeros((8, 128), u32), blk[:, kk * 128:(kk + 1) * 128])
            blk = jnp.concatenate([blk[:, :kk * 128], tl, blk[:, (kk + 1) * 128:]], axis=1)
            lhs_w = jnp.concatenate([lhs_w[:rg * 8], blk, lhs_w[(rg + 1) * 8:]], axis=0)

        def run(todo, src, scale, off):
            for pos, f in todo:
                r = min(int((pos - off) * scale * tiles), tiles - 1)
                t = f(src[r * 8:(r + 1) * 8, 0:128])
                if t is not None:
                    st["pending"].append(t)

        if not side:
            res = _dot(_unpack(lhs_w), rhs, dims)
        elif len(side) <= 2 and dims is NN and st["prev"] is not None:
            run(side, st["prev"], 1.0, 0.0)
            res = _dot(_unpack(lhs_w), rhs, dims)
        else:
            res = None
            for h in range(2):
                ks = slice(h * (D // 2), (h + 1) * (D // 2))
                part = _dot(_unpack(lhs_w[:, ks]), rhs[:, ks] if dims is NT else rhs[ks, :], dims)
                run([(p, f) for p, f in side if (p >= 0.5) == (h == 1)], part, 2.0, 0.5 * h)
                res = part if res is None else res + part
            st["done"] += st["pending"]
            st["pending"] = []
        st["prev"] = res
        return res

    def spread(q, k):
        items = [q.pop(0) for _ in range(min(k, len(q)))]
        return [(0.95 * j / len(items), f) for j, f in enumerate(items)]

    def ln_piece(i, c, tok=None):
        r0 = i * TM + c * CR
        xf = x_v[pl.ds(r0, CR), :].astype(f32)
        mean = gated(jnp.sum(xf, axis=1, keepdims=True), tok) * (1.0 / D)
        mb = _rb(mean)
        d = xf - mb
        dm = mean - mb
        var = jnp.sum(d * d, axis=1, keepdims=True) * (1.0 / D) - dm * dm
        rs = jnp.sum(d * st["wr"], axis=1, keepdims=True)
        inv = 1.0 / _rb(jnp.sqrt(_rb(_rb(var) + EPS_B)))
        r = _rb(rs * inv)
        packed = _pack(d * inv)
        xn32[pl.ds(r0 // 2, CR // 2), :] = packed
        ridx = lax.broadcasted_iota(i32, (CR, 1), 0) + r0
        if st["best"] is None:
            st["best"], st["bidx"] = r, ridx
        else:
            take = r > st["best"]
            st["best"] = jnp.where(take, r, st["best"])
            st["bidx"] = jnp.where(take, ridx, st["bidx"])
        return None if tok is None else _or_tiles(packed)

    def xw(i):
        return xn32[pl.ds(i * TM // 2, TM // 2), :]

    for c0 in range(X0):
        if c0 == 0:
            wr_cp.wait()
        x0s[c0].wait()
        kick(("x0", c0))
        if c0 == 0:
            st["wr"] = wr_v[...].astype(f32).reshape(1, D)
            one = (pltpu.bitcast(jnp.broadcast_to(st["wr"][:, 0:128], (8, 128)), i32) | 1) & 1
            st["big"] = pltpu.bitcast(one * 0x7F800000, f32)
            st["zero"] = pltpu.bitcast(jnp.concatenate([one - 1] * 8, axis=0), u32)
        for c in range(c0 * NLN // X0, (c0 + 1) * NLN // X0):
            ln_piece(0, c)

    pkb, vb = {}, {}
    kv = [None] * G
    zacc = [None] * G

    def K(i, g, side):
        pk = _phi(mm(xw(i), wk_v[:, g * 128:(g + 1) * 128], side))
        zp = jnp.sum(pk.reshape(TM // 8, 8, 128), axis=0)
        zacc[g] = zp if zacc[g] is None else zacc[g] + zp
        pkb[i, g] = pk.astype(bf16)

    def V(i, g, side):
        vb[i, g] = mm(xw(i), wv_v[:, g * 128:(g + 1) * 128], side).astype(bf16)

    def KV(i, g):
        if i < NB - 1:
            zero = jnp.concatenate([st["zero"]] * (TM // 128), axis=1)
            p = _dot(_unpack(pltpu.bitcast(pkb.pop((i, g)).T, u32) | zero), vb.pop((i, g)))
        else:
            p = _dot(pkb.pop((i, g)), vb.pop((i, g)), TN)
        kv[g] = p if kv[g] is None else kv[g] + p

    ys = dict(yv=None)
    rt = {}

    def col_bcast(dst, k0, row):
        for t in range(row.shape[1] // 128):
            dst[pl.ds(k0 + t * 128, 128), :] = jnp.broadcast_to(row[:, t * 128:(t + 1) * 128], (128, 128)).T

    def route():
        best, bidx = st["best"], st["bidx"]
        rmax = jnp.max(best)
        idx = jnp.minimum(jnp.min(jnp.where(best == rmax, bidx, S)), S - 1)
        idx16 = pl.multiple_of((idx // 16) * 16, 16)
        rt.update(rmax=rmax, idx=idx, idx16=idx16)
        slab = _unpack(xn32[pl.ds(pl.multiple_of(idx16 // 2, 8), 8), :]).astype(f32)
        pick = lax.broadcasted_iota(i32, (16, D), 0) == idx - idx16
        col_bcast(xb_v, 0, jnp.sum(jnp.where(pick, slab, 0.0), axis=0, keepdims=True))

    def mv_step(accs, b_ref, k0, nk, w_refs, c0, nc, tok=None):
        for kb in range(nk // KB):
            rows = pl.ds(k0 + kb * KB, KB)
            bt = jnp.concatenate([gated(b_ref[rows, :], tok)] * (nc // 128), axis=1)
            for j, w_ref in enumerate(w_refs):
                p = w_ref[rows, pl.ds(c0, nc)].astype(f32) * bt
                p = jnp.sum(p.reshape(KB // 8, 8, nc), axis=0)
                accs[j] = p if accs[j] is None else accs[j] + p

    def gu_slices(c):
        accs = [None, None]

        def fin(tok=None):
            gt = jnp.sum(accs[0], axis=0, keepdims=True)
            ut = jnp.sum(accs[1], axis=0, keepdims=True)
            col_bcast(hb_v, c * CH, _rb(gt * jax.nn.sigmoid(gt) * ut))

        return [functools.partial(mv_step, accs, xb_v, k0, SL, [wg_v, wu_v], c * CH, CH)
                for k0 in range(0, D, SL)] + [fin]

    def dn_step(k0, tok=None):
        accs = [ys["yv"]]
        mv_step(accs, hb_v, k0, SL // 2, [wd_v], 0, D, tok)
        ys["yv"] = accs[0]

    def wqt_slab(j):
        wt = pltpu.bitcast(wq_v[:, j * 128:(j + 1) * 128].T, u32)
        wqt32[j * 64:(j + 1) * 64, :] = wt | jnp.concatenate([st["zero"]] * G, axis=1)

    moe1 = [f for c in range(NC) for f in gu_slices(c)]
    moe2 = [functools.partial(dn_step, k0) for k0 in range(0, F, SL // 2)]
    n1 = -(-len(moe1) // (2 * G))
    n2 = -(-len(moe2) // NSLOT2)

    pend = []
    for i in range(NB):
        lastb = i == NB - 1
        lnq = [] if lastb else [functools.partial(ln_piece, i + 1, c) for c in range(NLN)]
        for g in range(G):
            if i == 0:
                for j, (g0, _) in enumerate(WSL):
                    if g == g0:
                        wks[j].wait()
                        if j > 0:
                            wvs[j].wait()
                        if g == 4:
                            x1s[0].wait()
                        if g == 6:
                            x1s[1].wait()
                        kick(("w", j))
            if i == 1 and g == 2:
                for j in range(2, NB):
                    xs[j].wait()
            if lastb and g == 0:
                wg_cp.wait()
                wu_cp.wait()
                wq_cp.wait()
                route()
            for m, MAT in enumerate((K, V)):
                if i == 0 and g == 0 and m == 1:
                    wvs[0].wait()
                if lastb:
                    side = spread(moe1, n1)
                    if m == 1:
                        wqt_slab(g)
                elif i == 0:
                    side = spread(lnq, NLN // 8) if g >= 4 else []
                elif i == 1:
                    side = spread(lnq, -(-len(lnq) // (2 * (G - g) - m))) if g >= 2 else []
                else:
                    side = spread(lnq, NLN // (2 * G))
                MAT(i, g, side)
            pend.append((i, g))
        assert not lnq
        if not lastb:
            while pend:
                KV(*pend.pop(0))
    assert not moe1

    idx, idx16, rmax = rt["idx"], rt["idx16"], rt["rmax"]
    same = lax.broadcasted_iota(i32, (128, 128), 0) // DH == lax.broadcasted_iota(i32, (128, 128), 1) // DH

    def Mp(g):
        kvb = jnp.where(same, kv[g], 0.0).astype(bf16)
        m32[g * 64:(g + 1) * 64, :] = _pack(_dot(kvb, wo_v[g * 128:(g + 1) * 128, :]))

    def ZC(g):
        z = jnp.sum(zacc[g], axis=0, keepdims=True)
        zc_v[g * 128:(g + 1) * 128, :] = jnp.broadcast_to(z, (128, 128)).T

    def Q(i, t):
        w0 = (i * TM + t * 128) // 2
        p = _phi(mm(wqt32[...], _unpack(xn32[w0:w0 + 64, :]), spread(moe2, 2 * n2), NT))
        tz = jnp.sum((p * zc_v[...]).reshape(H, DH // 8, 8, 128), axis=1)
        den = jnp.sum(tz, axis=1, keepdims=True) + 1e-6
        rc = pl.reciprocal(den, approx=True)
        rc = rc * (2.0 - den * rc)
        o = (p.reshape(H, DH, 128) * rc).reshape(D, 128)
        for g in range(G):
            ot = o[g * 128:(g + 1) * 128, :].astype(bf16)
            op32[w0:w0 + 64, g * 128:(g + 1) * 128] = pltpu.bitcast(ot.T, u32) | st["zero"]

    def OUT(i, g):
        cols = slice(g * 128, (g + 1) * 128)
        acc = mm(op32[pl.ds(i * TM // 2, TM // 2), :], _unpack(m32[:, cols]), spread(moe2, n2))
        res = (x_v[pl.ds(i * TM, TM), cols].astype(f32)
               + _unpack(xn32[pl.ds(i * TM // 2, TM // 2), cols]).astype(f32))
        out_v[pl.ds(i * TM, TM), cols] = (acc + res).astype(bf16)

    rr = lax.broadcasted_iota(i32, (16, D), 0)

    def patch(i, cols=slice(None)):
        slab = pl.multiple_of(jnp.clip(idx16, i * TM, (i + 1) * TM - 16), 16)
        cur = out_v[pl.ds(slab, 16), cols]
        upd = (cur.astype(f32) + ys["yg"][:, cols]).astype(bf16)
        out_v[pl.ds(slab, 16), cols] = jnp.where(rr[:, cols] + slab == idx, upd, cur)

    wo_cp.wait()
    wd_cp.wait()
    for g in range(G):
        ZC(g)
    for _ in range(4):
        KV(*pend.pop(0))
    Q(0, 0)
    while pend:
        KV(*pend.pop(0))
    Mp(0); Mp(1)
    Q(0, 1)
    Mp(2); Mp(3); Mp(4)
    Q(0, 2)
    Mp(5); Mp(6); Mp(7)
    Q(0, 3)

    for i in range(NB - 1):
        for t in range(4):
            Q(i + 1, t)
            OUT(i, 2 * t)
            OUT(i, 2 * t + 1)
        if i == 0:
            while moe2:
                moe2.pop(0)()
            gate = jax.nn.sigmoid(jnp.full((1, 1), rmax, f32))
            ys["yg"] = jnp.broadcast_to(jnp.sum(ys["yv"], axis=0, keepdims=True), (16, D)) * gate
        patch(i)
        outs[i].start()
    for g in range(G):
        OUT(NB - 1, g)
        patch(NB - 1, slice(g * 128, (g + 1) * 128))
        outs_last[g].start()
    for c in outs + outs_last:
        c.wait()
    assert not queue and not late


def make_kernel():
    any_spec = pl.BlockSpec(memory_space=pl.ANY)
    scratch = [
        pltpu.VMEM((S, D), bf16),
        pltpu.VMEM((S // 2, D), u32),
        pltpu.VMEM((D, D), bf16),
        pltpu.VMEM((D, D), bf16),
        pltpu.VMEM((D, D), bf16),
        pltpu.VMEM((D, D), bf16),
        pltpu.VMEM((D // 2, D), u32),
        pltpu.VMEM((S // 2, D), u32),
        pltpu.VMEM((D,), bf16),
        pltpu.VMEM((D, F), bf16),
        pltpu.VMEM((D, F), bf16),
        pltpu.VMEM((F, D), bf16),
        pltpu.VMEM((S, D), bf16),
        pltpu.VMEM((D, 128), f32),
        pltpu.VMEM((F, 128), f32),
        pltpu.VMEM((D // 2, D), u32),
        pltpu.VMEM((D, 128), f32),
        pltpu.SemaphoreType.DMA((X0,)),
        pltpu.SemaphoreType.DMA((NB,)),
        pltpu.SemaphoreType.DMA((len(WSL),)),
        pltpu.SemaphoreType.DMA((len(WSL),)),
        pltpu.SemaphoreType.DMA((6,)),
        pltpu.SemaphoreType.DMA((NB - 1 + G,)),
    ]

    def run(A_x, A_wqkv, A_wo, B_x, B_w_r, B_w_gate, B_w_up, B_w_down):
        del B_x
        out = pl.pallas_call(
            _kernel,
            out_shape=jax.ShapeDtypeStruct((S, D), bf16),
            in_specs=[any_spec] * 7,
            out_specs=any_spec,
            scratch_shapes=scratch,
            compiler_params=pltpu.CompilerParams(vmem_limit_bytes=120 * 2**20),
        )(A_x.reshape(S, D), A_wqkv, A_wo, B_w_r, B_w_gate, B_w_up, B_w_down)
        return out.reshape(1, S, D)
    return jax.jit(run)


_run = make_kernel()


@jax.jit
def pallas_parallel_sum__linear_attn_block__moe_arch_mod__prompt_kernel(
    A_x: jax.Array,
    A_wqkv: jax.Array,
    A_wo: jax.Array,
    B_x: jax.Array,
    B_w_r: jax.Array,
    B_w_gate: jax.Array,
    B_w_up: jax.Array,
    B_w_down: jax.Array,
):
    return _run(A_x, A_wqkv, A_wo, B_x, B_w_r, B_w_gate, B_w_up, B_w_down)
```
